```python
import jax
import jax.numpy as jnp

def _softmax(x, axis=-1):
    return jax.nn.softmax(x, axis=axis)
def _gelu(x):
    return jax.nn.gelu(x, approximate=True)
def _silu(x):
    return jax.nn.silu(x)
def _sigmoid(x):
    return jax.nn.sigmoid(x)
def _layernorm(x, axis=-1, eps=1e-5):
    m = jnp.mean(x, axis=axis, keepdims=True)
    v = jnp.var(x, axis=axis, keepdims=True)
    return (x - m) / jnp.sqrt(v + eps)
def _scatter_add(tgt, idx, src, axis=0):
    return tgt.at[idx].add(src)
def _segment_sum(src, seg, n):
    return jax.ops.segment_sum(src, seg, n)
class _Rng:
    def __init__(self, key):
        self._k = key
    def _next(self):
        self._k, sub = jax.random.split(self._k)
        return sub
    def normal(self, shape):
        return jax.random.normal(self._next(), shape, dtype=jnp.bfloat16)
    def randint(self, lo, hi, shape):
        return jax.random.randint(self._next(), shape, lo, hi, dtype=jnp.int32)
    def uniform(self, shape, lo=0.0, hi=1.0):
        return jax.random.uniform(self._next(), shape, jnp.bfloat16, lo, hi)
    def permutation(self, n):
        return jax.random.permutation(self._next(), n)


kernel_name = 'concat_heads__sliding_block_cached__compressed_kv_cla__decode'

def setup_inputs():
    _rng = _Rng(jax.random.key(int.from_bytes(__import__("os").urandom(4), "little")))
    _w = (lambda a: (lambda t: t.astype(jnp.bfloat16) if jnp.issubdtype(t.dtype, jnp.floating) else t)(jnp.asarray(a)))
    def _A_setup():
        B, Sq, D = 4, 1, 512
        Hq, Hkv, Sk, Dh = 32, 32, 4096, 128
        assert Hq % Hkv == 0, (Hq, Hkv)
        return {
            "x": _w((lambda *s: _rng.normal(s) * 0.05)(B, Sq, D)),
            "k_cache": _w((lambda *s: _rng.normal(s) * 0.05)(B, Hkv, Sk, Dh)),
            "v_cache": _w((lambda *s: _rng.normal(s) * 0.05)(B, Hkv, Sk, Dh)),
            "wq": _w((lambda *s: _rng.normal(s) * 0.05)(D, Hq * Dh) * (D ** -0.5)),
            "wo": _w((lambda *s: _rng.normal(s) * 0.05)(Hq * Dh, D) * ((Hq * Dh) ** -0.5)),
        }
    _A_in = _A_setup()

    def _B_setup():
        B, H, Sq, Sk, D, M = 4, 32, 1, 4096, 128, 512
        Dc = 4 * D
        return {
            "x": _w((lambda *s: _rng.normal(s) * 0.05)(B, Sq, M)),
            "c_kv": _w((lambda *s: _rng.normal(s) * 0.05)(B, Sk, Dc)),
            "w_q": _w((lambda *s: _rng.normal(s) * 0.05)(M, H, D) * (M ** -0.5)),
            "w_uk": _w((lambda *s: _rng.normal(s) * 0.05)(Dc, H, D) * (Dc ** -0.5)),
            "w_uv": _w((lambda *s: _rng.normal(s) * 0.05)(Dc, H, D) * (Dc ** -0.5)),
            "w_o": _w((lambda *s: _rng.normal(s) * 0.05)(H, D, M) * ((H * D) ** -0.5)),
        }
    _B_in = _B_setup()

    return {
        "A_x": _A_in["x"],
        "A_k_cache": _A_in["k_cache"],
        "A_v_cache": _A_in["v_cache"],
        "A_wq": _A_in["wq"],
        "A_wo": _A_in["wo"],
        "B_x": _B_in["x"],
        "B_c_kv": _B_in["c_kv"],
        "B_w_q": _B_in["w_q"],
        "B_w_uk": _B_in["w_uk"],
        "B_w_uv": _B_in["w_uv"],
        "B_w_o": _B_in["w_o"],
    }

def reference(A_x, A_k_cache, A_v_cache, A_wq, A_wo, B_x, B_c_kv, B_w_q, B_w_uk, B_w_uv, B_w_o):
    def _A_ref(x, k_cache, v_cache, wq, wo):
        B, Sq, D = x.shape
        Hq, Dh = 32, 128
        Hkv, Sk = k_cache.shape[1], k_cache.shape[2]
        W = min(4096, max(256, Sk // 4))
        rep = Hq // Hkv
        q = (lambda x, *d: x.transpose(*d))((x @ wq).reshape(B, Sq, Hq, Dh), 0, 2, 1, 3)
        k = jnp.repeat(k_cache[:, :, Sk - W:, :], rep, axis=1)
        v = jnp.repeat(v_cache[:, :, Sk - W:, :], rep, axis=1)
        scores = jnp.einsum("bhqd,bhkd->bhqk", q, k) * (Dh ** -0.5)
        p = _softmax(scores, axis=-1)
        o = jnp.einsum("bhqk,bhkd->bhqd", p, v)
        return (lambda x, *d: x.transpose(*d))(o, 0, 2, 1, 3).reshape(B, Sq, Hq * Dh) @ wo

    def _B_ref(x, c_kv, w_q, w_uk, w_uv, w_o):
        B, Sq, M = x.shape[0], x.shape[1], x.shape[2]
        Sk = c_kv.shape[1]
        H, D = w_q.shape[1], w_q.shape[2]
        q = jnp.einsum("bqm,mhd->bhqd", x, w_q)
        k = jnp.einsum("bkc,chd->bhkd", c_kv, w_uk)
        v = jnp.einsum("bkc,chd->bhkd", c_kv, w_uv)
        scores = jnp.einsum("bhqd,bhkd->bhqk", q, k) * (D ** -0.5)
        off = Sk - Sq
        qi = jnp.arange(Sq)[:, None]
        kj = jnp.arange(Sk)[None, :]
        cmask = kj <= (qi + off)
        scores = jnp.where(cmask[None, None], scores, -1e9)
        p = _softmax(scores, axis=-1)
        ctx = jnp.einsum("bhqk,bhkd->bhqd", p, v)
        return jnp.einsum("bhqd,hdm->bqm", ctx, w_o)

    a = _A_ref(A_x, A_k_cache, A_v_cache, A_wq, A_wo)
    b = _B_ref(B_x, B_c_kv, B_w_q, B_w_uk, B_w_uv, B_w_o)
    return jnp.concatenate([a, b], axis=-1)
```

```python
import functools
import jax
import jax.numpy as jnp
from jax import lax
from jax.experimental import pallas as pl
from jax.experimental.pallas import tpu as pltpu

NB, NH, DH, DM, SK = 4, 32, 128, 512, 4096
WIN = 1024
W0 = SK - WIN
STEPS = 16
RING = 8
F32, BF16 = jnp.float32, jnp.bfloat16
NT = (((1,), (1,)), ((), ()))


def build(look=6, d_idle=100, d_q=0, d_bq=0, d_abs=0, d_s=0, d_pv=0, d_k=0, d_v=0, d_ctx=0, d_out=0,
          mul=9, diag=1, dma=True, compute=True):
    def kern(xa_h, k_h, v_h, wq_h, wo_h, xb_h, c_h, bwq_h, wuk_h, wuv_h, bwo_h, o_ref,
             xa_v, xb_v, k_v, v_v, wq_v, wo_v, c_v, bwq_v, wuk_v, wuv_v, bwo_v,
             qa_s, qb_s, qabs_s, sb_s, cc_s, sa_s, oa_s, ob_s, sems, xsem):

        def rows_stream(src, dst, rpb, blk):
            def piece(s, j):
                sb, db = blk(s, j)
                n = rpb if j < 3 else rpb // 2
                half = rpb // 2 if j == 4 else 0
                so = pl.multiple_of(sb * rpb + half, n)
                do = pl.multiple_of(db * rpb + half, n)
                return src.at[pl.ds(so, n)], dst.at[pl.ds(do, n)]
            return piece

        def order(s, j):
            t = s & 15
            return t * 3 + j if j < 3 else 48 + t

        def flat_blk(s, j):
            b = (s >> 4) * 64 + ((order(s, j) * mul) & 63)
            return b, b

        def win_blk(s, j):
            t = s & 15
            if j < 3:
                n = t * 3 + j
                h = n & 15
                p = n >> 4
                if diag:
                    p = p + h
                    p = p - 3 * ((p * 11) >> 5)
            else:
                h = (t + 8) & 15
                p = 3
            h = (s >> 4) * 16 + h
            return h * 16 + 12 + p, h * 4 + p

        def last_head(s, second):
            t = ((s & 15) * 5) & 15
            return t + 16 if second else t

        def last_blk(s, j):
            b = last_head(s, j in (1, 3, 4)) * 2 + (1 if j >= 2 else 0)
            return b, b

        def wq_piece(s, j):
            r = pl.multiple_of(flat_blk(s, j)[0] * 8, 8)
            c = slice(None) if j < 3 else pl.ds((j - 3) * 2048, 2048)
            return wq_h.at[pl.ds(r, 8), c], wq_v.at[pl.ds(r, 8), c]

        st_bwq = rows_stream(bwq_h.bitcast(jnp.uint32), bwq_v, 128, flat_blk)
        st_wuk = rows_stream(wuk_h.bitcast(jnp.uint32), wuk_v, 128, flat_blk)
        st_wuv = rows_stream(wuv_h.bitcast(jnp.uint32), wuv_v, 128, flat_blk)
        st_c = rows_stream(c_h, c_v, 64, flat_blk)
        st_k = rows_stream(k_h, k_v, 256, win_blk)
        st_v = rows_stream(v_h, v_v, 256, win_blk)
        st_wo = rows_stream(wo_h, wo_v, 64, flat_blk)
        st_bwo = rows_stream(bwo_h, bwo_v, 64, last_blk)

        def copy(stream, s, j):
            src, dst = stream(s, j)
            return pltpu.make_async_copy(src, dst, sems.at[s & (RING - 1)])

        def begin(stream, s, js):
            for j in js:
                copy(stream, s, j).start(priority=1 if j < 3 else 0)

        def issue(cur, nxt, s, js):
            if not dma:
                return
            t = s + look
            for lst, inside, tt in ((cur, t < STEPS, t), (nxt, t >= STEPS, t - STEPS)):
                for cond, stream, unit in lst:
                    c = inside if cond is True else jnp.logical_and(inside, cond)
                    pl.when(c)(functools.partial(begin, stream, unit * STEPS + tt, js))

        def arrive(stream, s):
            if dma:
                for j in range(5):
                    copy(stream, s, j).wait()

        def phase(cur, nxt, body, init=0, delay=0, lo=0, hi=STEPS):
            def it(s, carry):
                arrive(st_k, s)
                issue(cur, nxt, s, (0, 1, 2, 3))
                if compute:
                    carry = body(s, carry)
                if delay:
                    pl.delay(delay)
                issue(cur, nxt, s, (4,))
                return carry
            return lax.fori_loop(lo, hi, it, init)

        if dma:
            def first(s, c):
                begin(wq_piece, s, range(5))
                return c
            lax.fori_loop(0, look, first, 0)
        xcp = [pltpu.make_async_copy(xa_h, xa_v, xsem.at[0]), pltpu.make_async_copy(xb_h, xb_v, xsem.at[1])]
        for cp in xcp:
            cp.start(priority=1)

        phase([(True, wq_piece, 0)], [(True, st_bwq, 0)], lambda s, c: c, delay=d_idle)
        for cp in xcp:
            cp.wait()

        def q_body(s, c):
            w = wq_v[:, pl.ds(pl.multiple_of(s * 256, 256), 256)]
            q = jnp.dot(xa_v[...], w, preferred_element_type=F32)
            for i in range(2):
                qa_s[pl.ds(2 * s + i, NB, stride=NH), :] = q[:, i * DH:(i + 1) * DH]
            return c
        phase([(True, st_bwq, 0)], [(True, st_wuk, 0)], q_body, delay=d_q)

        def head_pair(w_v, s):
            w = w_v[pl.ds(s, DM, stride=NH // 2), :]
            lo = pltpu.bitcast(w << 16, F32).astype(BF16)
            hi = pltpu.bitcast(w & jnp.uint32(0xFFFF0000), F32).astype(BF16)
            return lo, hi

        def bq_body(s, c):
            for i, w in enumerate(head_pair(bwq_v, s)):
                qb_s[2 * s + i] = jnp.dot(xb_v[...], w, preferred_element_type=F32)
            return c
        phase([(True, st_wuk, 0)], [(True, st_c, 0)], bq_body, delay=d_bq)

        def abs_body(s, c):
            for i, w in enumerate(head_pair(wuk_v, s)):
                r = lax.dot_general(qb_s[2 * s + i].astype(BF16), w, NT, preferred_element_type=F32)
                for t in range(4):
                    qabs_s[t, pl.ds(2 * s + i, NB, stride=NH), :] = r[:, t * 128:(t + 1) * 128]
            return c
        phase([(True, st_c, 0)], [(True, st_c, 1)], abs_body, delay=d_abs)

        scale = DH ** -0.5

        def latent(b, c):
            cur = [(b < NB - 1, st_c, b + 1), (b == NB - 1, st_k, 0)]
            nxt = [(b < NB - 2, st_c, b + 2), (b == NB - 2, st_k, 0), (b == NB - 1, st_v, 0)]
            r0 = pl.multiple_of(b * NH, NH)
            q = jnp.concatenate([qabs_s[t, pl.ds(r0, NH), :] for t in range(4)], axis=1).astype(BF16)

            def keys(s):
                return c_v[pl.ds(pl.multiple_of(b * SK + s * 512, 512), 512), :]

            def s_body(s, m):
                sc = lax.dot_general(q, keys(s), NT, preferred_element_type=F32) * scale
                sb_s[s] = sc
                for t in range(4):
                    m = jnp.maximum(m, sc[:, t * 128:(t + 1) * 128])
                return m
            m = phase(cur, nxt, s_body, jnp.full((NH, 128), -jnp.inf, F32), d_s, 0, 8)
            m = jnp.max(m, axis=1, keepdims=True)

            def pv_body(s, carry):
                l, acc = carry
                p = jnp.exp(sb_s[s - 8] - m)
                for t in range(4):
                    l = l + p[:, t * 128:(t + 1) * 128]
                return l, acc + jnp.dot(p.astype(BF16), keys(s - 8), preferred_element_type=F32)
            l, acc = phase(cur, nxt, pv_body, (jnp.zeros((NH, 128), F32), jnp.zeros((NH, DM), F32)), d_pv, 8, 16)
            acc = acc / jnp.sum(l, axis=1, keepdims=True)
            for t in range(4):
                cc_s[t, pl.ds(r0, NH), :] = acc[:, t * 128:(t + 1) * 128]
            return c
        lax.fori_loop(0, NB, latent, 0)

        NU = NB * NH // 16

        def window(u, c):
            def rows(s):
                return pl.ds(pl.multiple_of((u * 16 + s) * WIN, WIN), WIN)

            def k_body(s, c):
                q = jnp.broadcast_to(qa_s[pl.ds(u * 16 + s, 1), :], (8, DH)).astype(BF16)
                sc = lax.dot_general(q, k_v[rows(s), :], NT, preferred_element_type=F32)
                sa_s[pl.ds(s, 1), :] = sc[0:1]
                return c
            phase([(True, st_v, u)], [(u < NU - 1, st_k, u + 1), (u == NU - 1, st_wuv, 0)], k_body, delay=d_k)
            if compute:
                sc = sa_s[...] * scale
                p = jnp.exp(sc - jnp.max(sc, axis=1, keepdims=True))
                sa_s[...] = p / jnp.sum(p, axis=1, keepdims=True)

            def v_body(s, c):
                p = jnp.broadcast_to(sa_s[pl.ds(s, 1), :], (8, WIN)).astype(BF16)
                o = jnp.dot(p, v_v[rows(s), :], preferred_element_type=F32)
                oa_s[pl.ds(u * 16 + s, 1), :] = o[0:1]
                return c
            phase([(u < NU - 1, st_k, u + 1), (u == NU - 1, st_wuv, 0)],
                  [(u < NU - 1, st_v, u + 1), (u == NU - 1, st_wo, 0)], v_body, delay=d_v)
            return c
        lax.fori_loop(0, NU, window, 0)

        def ctx_body(s, c):
            for i, w in enumerate(head_pair(wuv_v, s)):
                cc = jnp.concatenate([cc_s[t, pl.ds(2 * s + i, NB, stride=NH), :] for t in range(4)], axis=1)
                ob_s[2 * s + i] = jnp.dot(cc.astype(BF16), w, preferred_element_type=F32)
            return c
        phase([(True, st_wo, 0)], [(True, st_bwo, 0)], ctx_body, delay=d_ctx)

        def out_it(s, carry):
            ya, yb = carry
            if compute:
                for i in range(2):
                    h = 2 * s + i
                    o = oa_s[pl.ds(h, NB, stride=NH), :].astype(BF16)
                    ya = ya + jnp.dot(o, wo_v[pl.ds(pl.multiple_of(h * DH, DH), DH), :], preferred_element_type=F32)
            arrive(st_k, s)
            issue([(True, st_bwo, 0)], [], s, (0, 1, 2, 3))
            if compute:
                for i in range(2):
                    h = last_head(s, i)
                    yb = yb + jnp.dot(ob_s[h].astype(BF16), bwo_v[pl.ds(pl.multiple_of(h * DH, DH), DH), :],
                                      preferred_element_type=F32)
            if d_out:
                pl.delay(d_out)
            issue([(True, st_bwo, 0)], [], s, (4,))
            return ya, yb
        z = jnp.zeros((NB, DM), F32)
        ya, yb = lax.fori_loop(0, STEPS, out_it, (z, z))
        o_ref[:, 0:DM] = ya.astype(BF16)
        o_ref[:, DM:2 * DM] = yb.astype(BF16)

    @jax.jit
    def f(A_x, A_k_cache, A_v_cache, A_wq, A_wo, B_x, B_c_kv, B_w_q, B_w_uk, B_w_uv, B_w_o):
        vm = pltpu.VMEM
        out = pl.pallas_call(
            kern,
            out_shape=jax.ShapeDtypeStruct((NB, 2 * DM), BF16),
            in_specs=[pl.BlockSpec(memory_space=pl.ANY)] * 11,
            out_specs=pl.BlockSpec(memory_space=vm),
            scratch_shapes=[
                vm((NB, DM), BF16), vm((NB, DM), BF16),
                vm((NB * NH * WIN, DH), BF16), vm((NB * NH * WIN, DH), BF16),
                vm((DM, NH * DH), BF16), vm((NH * DH, DM), BF16), vm((NB * SK, DM), BF16),
                vm((DM * NH // 2, DH), jnp.uint32), vm((DM * NH // 2, DH), jnp.uint32), vm((DM * NH // 2, DH), jnp.uint32),
                vm((NH * DH, DM), BF16),
                vm((NB * NH, DH), F32), vm((NH, NB, DH), F32), vm((4, NB * NH, 128), F32),
                vm((8, NH, 512), F32), vm((4, NB * NH, 128), F32), vm((16, WIN), F32),
                vm((NB * NH, DH), F32), vm((NH, NB, DH), F32),
                pltpu.SemaphoreType.DMA((RING,)), pltpu.SemaphoreType.DMA((2,)),
            ],
            compiler_params=pltpu.CompilerParams(vmem_limit_bytes=120 * 1024 * 1024, disable_bounds_checks=True),
        )(A_x.reshape(NB, DM), A_k_cache.reshape(-1, DH), A_v_cache.reshape(-1, DH), A_wq, A_wo,
          B_x.reshape(NB, DM), B_c_kv.reshape(-1, DM), B_w_q.reshape(-1, DH), B_w_uk.reshape(-1, DH),
          B_w_uv.reshape(-1, DH), B_w_o.reshape(-1, DM))
        return out.reshape(NB, 1, 2 * DM)
    return f


pallas_concat_heads__sliding_block_cached__compressed_kv_cla__decode_kernel = build()
```

```python
import contextlib
import functools
import jax
import jax.numpy as jnp
from jax import lax
from jax.experimental import pallas as pl
from jax.experimental.pallas import tpu as pltpu

NB, NH, DH, DM, SK = 4, 32, 128, 512, 4096
WIN = 1024
F32, BF16, U32 = jnp.float32, jnp.bfloat16, jnp.uint32
NT = (((1,), (1,)), ((), ()))
RING = 4
SCALE = DH ** -0.5
T_WQ, T_BWQ, T_WUK, T_C, T_WUV, T_KV, T_BWO, T_WO, T_END = 0, 8, 16, 24, 56, 64, 192, 200, 208

P2 = "e0 e1 w0 w1 w2 E0 p0 p1 p2 c E1 w3 w4 w5 E2 p3 p4 p5 c E3"
P4 = "e0 e1 w0 w1 w2 E0 p0 p1 p2 c E1 c w3 w4 w5 E2 p3 p4 p5 c E3 c"
PI = "e0 e1 w0 E0 p0 w1 p1 w2 E1 p2 w3 E2 p3 w4 p4 w5 E3 p5"
PO = "e0 e1 w0 E0 p0 c E1 w1 p1 w2 p2 c w3 E2 p3 c w4 p4 c E3 w5 p5 c"
PA = "w0 E0 p0 e0 c w1 p1 w2 E1 p2 w3 E2 p3 e1 c w4 p4 w5 E3 p5"
PB = "w0 E0 e0 c w1 w2 E1 p0 p1 p2 w3 E2 e1 c w4 w5 E3 p3 p4 p5"
PC = "w0 E0 e0 p0 p1 p2 c w1 w2 E1 w3 E2 e1 p3 p4 p5 c w4 w5 E3"
PD = "w0 E0 e0 p0 c w1 w2 E1 p1 p2 w3 E2 e1 p3 c w4 w5 E3 p4 p5"
PE = "w0 p0 w1 E0 e0 p1 c w2 w3 E1 p2 p3 w4 E2 e1 p4 c w5 p5 E3"
PF = "w0 E0 p0 w1 E1 e0 p1 c w2 w3 E2 p2 p3 w4 E3 e1 p4 c w5 p5"
PG = "w0 E0 e0 p0 p1 p2 c w1 E1 w2 w3 E2 e1 p3 p4 p5 c w4 E3 w5"
PO = "e0 e1 w0 E0 p0 p1 p2 w1 w2 E1 c w3 E2 p3 p4 p5 c w4 c w5 E3 c"


def build(L=3, rot=16, compute=True, fs=(0, 4, 7, 3, 6, 2, 2, 6, 2, 6), ks=(0, 0, -2, -2, -4, -4, -5, -5, -5, -5),
          ls=(0, 4, 0, 4, 0, 4, 0, 4, 0, 4), M=33, bc=False, only=None, flags=None, plans={}, P=PG, pitch=24, scopes=False):
    pn = dict(idle=PI, q=P, bq=P, ab=P, lat=P, ctx=P, kv=P, out=PO)
    pn.update(plans)
    if not compute:
        pn = {k: pn["idle"] for k in pn}

    def kern(xa_h, k_h, v_h, wq_h, wo_h, xb_h, c_h, bwq_h, wuk_h, wuv_h, bwo_h, o_ref,
             xa_v, xb_v, k_v, v_v, wq_v, wo_v, c_v, bwq_v, wuk_v, wuv_v, bwo_v,
             qa_s, qb_s, qabs_s, sb_s, cc_s, oa_s, ob_s, lo_sem, hi_sem, x_sem):

        class Stream:
            def __init__(self, first, last, refs, rows, rot, place, steps):
                self.first, self.last, self.refs, self.rows, self.rot = first, last, refs, rows, rot
                self.place, self.steps = place, steps

            def copy(self, x, j, off, size, sem, wrap=False):
                src, dst = self.refs[j & 1]
                u = self.rows // 16
                so, do = self.place(x - self.first, self.steps[j], j & 1, self.rows, off * u // 16, wrap)
                n = size * u // 16
                dst = dst.at[pl.ds(pl.multiple_of(do, u), n)]
                if dst.shape[1:] != src.shape[1:]:
                    dst = dst.at[:, pl.ds(0, src.shape[1])]
                return pltpu.make_async_copy(src.at[pl.ds(pl.multiple_of(so, u), n)], dst, sem)

            def page(self, x, j):
                return self.copy(x, j, self.rot + 32 + 64 * (j >> 1), 64, lo_sem.at[(x & (RING - 1)) * 6 + j])

            def edge(self, x, j):
                off, sem = self.rot + 224 * (j >> 1), hi_sem.at[(x & (RING - 1)) * 2 + (j >> 1)]
                if self.rot and j == 3:
                    return [self.copy(x, 6 + j, off, 256 - off, sem),
                            self.copy(x, 6 + j, 256, off + 32 - 256, sem, True)]
                return [self.copy(x, 6 + j, off, 32, sem)]

        def flat(t, step, side, rows, off, wrap):
            o = ((t + step + wrap) & 7) * (2 * rows) + (0 if wrap else side * rows + off)
            return o, o

        def flat_c(t, step, side, rows, off, wrap):
            o = (((t + step + wrap) & 7) + (t & -8)) * (2 * rows) + (0 if wrap else side * rows + off)
            return o, o

        def window(t, step, side, rows, off, wrap):
            h = (t * M + step * M) & 127
            return h * (4 * rows) + (3 * rows + off), h * rows + off

        def both(src, dst):
            return ((src, dst), (src, dst))

        st_wq = Stream(T_WQ, T_BWQ, both(wq_h, wq_v), 128, 0, flat, fs)
        st_kv = Stream(T_KV, T_BWO, ((k_h.bitcast(U32), k_v), (v_h.bitcast(U32), v_v)), 512, 0, window, ks)
        streams = [
            st_wq,
            Stream(T_BWQ, T_WUK, both(bwq_h.bitcast(U32), bwq_v), 32, rot, flat, fs),
            Stream(T_WUK, T_C, both(wuk_h.bitcast(U32), wuk_v), 32, rot, flat, fs),
            Stream(T_C, T_WUV, both(c_h, c_v), 256, rot, flat_c, fs),
            Stream(T_WUV, T_KV, both(wuv_h.bitcast(U32), wuv_v), 32, rot, flat, fs),
            st_kv,
            Stream(T_BWO, T_WO, both(bwo_h, bwo_v), 256, rot, flat, fs),
            Stream(T_WO, T_END, both(wo_h, wo_v), 256, 0, flat, ls),
        ]

        def each(lo, hi, x, fn):
            for st in streams:
                if st.last <= lo or st.first >= hi:
                    continue
                conds = ([x >= st.first] if st.first > lo else []) + ([x < st.last] if st.last < hi else [])
                if conds:
                    pl.when(functools.reduce(jnp.logical_and, conds))(functools.partial(fn, st))
                else:
                    fn(st)

        def start_edge(st, x, j):
            for cp in st.edge(x, j):
                cp.start()

        def run(lo, hi, name, body=None, init=0):
            def it(g, carry):
                x = g + L
                on = body is not None and compute and (only is None or name in only)
                segs = body(g, carry) if on else iter(())
                for op in pn[name].split():
                    if op[0] == "e":
                        whole = k_v.at[pl.ds(0, 128)]
                        pltpu.make_async_copy(whole, whole, hi_sem.at[(g & (RING - 1)) * 2 + int(op[1])]).wait()
                    elif op == "c":
                        carry = next(segs, carry)
                    elif op[0] == "w":
                        st_kv.page(g, int(op[1])).wait()
                    elif op[0] == "p":
                        each(lo + L, hi + L, x, lambda st, j=int(op[1]): st.page(x, j).start(priority=1))
                    else:
                        each(lo + L, hi + L, x, lambda st, j=int(op[1]): start_edge(st, x, j))
                for carry in segs:
                    pass
                return carry
            with jax.named_scope("ph_" + name) if scopes else contextlib.nullcontext():
                return lax.fori_loop(lo, hi, it, init)

        def first(x, c):
            for j in range(6):
                st_wq.page(x, j).start(priority=1)
            for j in range(4):
                start_edge(st_wq, x, j)
            return c
        lax.fori_loop(0, L, first, 0)
        xcp = [pltpu.make_async_copy(xa_h, xa_v, x_sem.at[0]), pltpu.make_async_copy(xb_h, xb_v, x_sem.at[1])]
        for cp in xcp:
            cp.start(priority=1)
        run(0, T_BWQ, "idle")
        for cp in xcp:
            cp.wait()

        def split(name, i):
            return pn[name].count("c") == 4 or i & 1

        def q_body(g, c):
            for i in range(4):
                h = (g - T_BWQ) * 4 + i
                w = jnp.concatenate([wq_v[r * NH + h] for r in range(DM // 8)], axis=0)
                qa_s[pl.ds(h, NB, stride=NH), :] = jnp.dot(xa_v[...], w, preferred_element_type=F32)
                if split("q", i):
                    yield c
        run(T_BWQ, T_WUK, "q", q_body)

        def head_pairs(w_v, t):
            for i in range(2):
                w = w_v.reshape(DM * pitch, DH)[pl.ds(2 * t + i, DM, stride=pitch), :]
                yield 4 * t + 2 * i, pltpu.bitcast(w << 16, F32).astype(BF16)
                yield 4 * t + 2 * i + 1, pltpu.bitcast(w & jnp.uint32(0xFFFF0000), F32).astype(BF16)

        def bq_body(g, c):
            for i, (h, w) in enumerate(head_pairs(bwq_v, g - T_WUK)):
                qb_s[h] = jnp.dot(xb_v[...], w, preferred_element_type=F32)
                if split("bq", i):
                    yield c
        run(T_WUK, T_C, "bq", bq_body)

        def abs_body(g, c):
            for i, (h, w) in enumerate(head_pairs(wuk_v, g - T_C)):
                r = lax.dot_general(qb_s[h].astype(BF16), w, NT, preferred_element_type=F32)
                for t in range(4):
                    qabs_s[t, pl.ds(h, NB, stride=NH), :] = r[:, t * 128:(t + 1) * 128]
                if split("ab", i):
                    yield c
        run(T_C, T_C + 8, "ab", abs_body)

        def lat_keys(t):
            return c_v[pl.ds(pl.multiple_of(t * 512, 512), 512), :]

        def lat_scores(t):
            r0 = pl.multiple_of((t >> 3) * NH, NH)
            q = jnp.concatenate([qabs_s[i, pl.ds(r0, NH), :] for i in range(4)], axis=1).astype(BF16)
            sb_s[...] = lax.dot_general(q, lat_keys(t), NT, preferred_element_type=F32) * SCALE

        def lat_body(g, carry):
            m, l = carry
            t = g - (T_C + 8)
            r0 = pl.multiple_of((t >> 3) * NH, NH)
            fresh = (t & 7) == 0
            m = jnp.where(fresh, -jnp.inf, m)
            s0 = sb_s[...]
            m_new = jnp.maximum(m, jnp.max(s0, axis=1, keepdims=True))
            alpha = jnp.exp(m - m_new)
            p = jnp.exp(s0 - m_new)
            l = jnp.where(fresh, 0.0, alpha * l) + jnp.sum(p, axis=1, keepdims=True)
            p = p.astype(BF16)
            lat_scores(jnp.minimum(t + 1, 31))
            yield carry
            pv = jnp.dot(p, lat_keys(t), preferred_element_type=F32)
            norm = jnp.where((t & 7) == 7, 1.0 / l, 1.0)
            for i in range(4):
                acc = cc_s[i, pl.ds(r0, NH), :]
                cc_s[i, pl.ds(r0, NH), :] = (alpha * acc + pv[:, i * 128:(i + 1) * 128]) * norm
            yield m_new, l
        if compute:
            cc_s[...] = jnp.zeros(cc_s.shape, F32)
            lat_scores(0)
        run(T_C + 8, T_KV, "lat", lat_body, (jnp.zeros((NH, 1), F32), jnp.zeros((NH, 1), F32)))

        def ctx_body(g, c):
            for i, (h, w) in enumerate(head_pairs(wuv_v, g - T_KV)):
                cc = jnp.concatenate([cc_s[t, pl.ds(h, NB, stride=NH), :] for t in range(4)], axis=1)
                ob_s[h] = jnp.dot(cc.astype(BF16), w, preferred_element_type=F32)
                if split("ctx", i):
                    yield c
        run(T_KV, T_KV + 8, "ctx", ctx_body)

        def kv_rows(ref, h):
            return pltpu.bitcast(ref[pl.ds(pl.multiple_of(h * 512, 512), 512), :], BF16)

        def kv_scores(i):
            h = (i * M) & 127
            q = jnp.broadcast_to(qa_s[pl.ds(h, 1), :], (8, DH)).astype(BF16)
            return lax.dot_general(q, kv_rows(k_v, h), NT, preferred_element_type=F32) * SCALE

        def kv_body(g, s0):
            i = g - (T_KV + 8)
            h = (i * M) & 127
            p = jnp.exp(s0 - jnp.max(s0, axis=1, keepdims=True))
            norm = 1.0 / jnp.sum(p, axis=1, keepdims=True)
            p = p.astype(BF16)
            s1 = kv_scores(jnp.minimum(i + 1, 127))
            yield s0
            o = jnp.dot(p, kv_rows(v_v, h), preferred_element_type=F32) * norm
            oa_s[pl.ds(h, 1), :] = o[0:1]
            t = i & 31
            yield s1
        run(T_KV + 8, T_WO, "kv", kv_body, kv_scores(0) if compute else 0)

        def out_body(g, carry):
            ya, yb = carry
            t = g - T_WO
            for i in range(4):
                h = 4 * t + i
                yb = yb + jnp.dot(ob_s[h].astype(BF16), bwo_v[pl.ds(pl.multiple_of(h * DH, DH), DH), :],
                                  preferred_element_type=F32)
            for i in range(4):
                h = ((t + 4 * (i & 1)) & 7) * 4 + 2 * (i & 1) + (i >> 1)
                o = oa_s[pl.ds(h, NB, stride=NH), :].astype(BF16)
                ya = ya + jnp.dot(o, wo_v[pl.ds(pl.multiple_of(h * DH, DH), DH), :], preferred_element_type=F32)
                yield ya, yb
        z = jnp.zeros((NB, DM), F32)
        ya, yb = run(T_WO, T_END, "out", out_body, (z, z))
        o_ref[:, 0:DM] = ya.astype(BF16)
        o_ref[:, DM:2 * DM] = yb.astype(BF16)

    @jax.jit
    def f(A_x, A_k_cache, A_v_cache, A_wq, A_wo, B_x, B_c_kv, B_w_q, B_w_uk, B_w_uv, B_w_o):
        vm = pltpu.VMEM
        wq = A_wq.reshape(DM // 8, 8, NH, DH).transpose(0, 2, 1, 3).reshape(DM // 8 * NH, 8, DH)
        out = pl.pallas_call(
            kern,
            out_shape=jax.ShapeDtypeStruct((NB, 2 * DM), BF16),
            in_specs=[pl.BlockSpec(memory_space=pl.ANY)] * 11,
            out_specs=pl.BlockSpec(memory_space=vm),
            scratch_shapes=[
                vm((NB, DM), BF16), vm((NB, DM), BF16),
                vm((NB * NH * WIN // 2, DH), U32), vm((NB * NH * WIN // 2, DH), U32),
                vm((DM // 8 * NH, 8, DH), BF16), vm((NH * DH, DM), BF16), vm((NB * SK, DM), BF16),
                vm((DM, pitch, DH), U32), vm((DM, pitch, DH), U32), vm((DM, pitch, DH), U32),
                vm((NH * DH, DM), BF16),
                vm((NB * NH, DH), F32), vm((NH, NB, DH), F32), vm((4, NB * NH, 128), F32),
                vm((NH, 512), F32), vm((4, NB * NH, 128), F32), vm((NB * NH, DH), F32), vm((NH, NB, DH), F32),
                pltpu.SemaphoreType.DMA((RING * 6,)), pltpu.SemaphoreType.DMA((RING * 2,)), pltpu.SemaphoreType.DMA((2,)),
            ],
            compiler_params=pltpu.CompilerParams(vmem_limit_bytes=120 * 1024 * 1024, disable_bounds_checks=not bc, disable_semaphore_checks=True, flags=flags),
        )(A_x.reshape(NB, DM), A_k_cache.reshape(-1, DH), A_v_cache.reshape(-1, DH), wq, A_wo,
          B_x.reshape(NB, DM), B_c_kv.reshape(-1, DM), B_w_q, B_w_uk,
          B_w_uv, B_w_o.reshape(-1, DM))
        return out.reshape(NB, 1, 2 * DM)
    return f


pallas_concat_heads__sliding_block_cached__compressed_kv_cla__decode_kernel = build()
```

```python
import contextlib
import functools
import jax
import jax.numpy as jnp
from jax import lax
from jax.experimental import pallas as pl
from jax.experimental.pallas import tpu as pltpu

NB, NH, DH, DM, SK = 4, 32, 128, 512, 4096
WIN = 1024
F32, BF16, U32 = jnp.float32, jnp.bfloat16, jnp.uint32
NT = (((1,), (1,)), ((), ()))
RING = 4
SCALE = DH ** -0.5
T_WQ, T_BWQ, T_WUK, T_C, T_WUV, T_KV, T_BWO, T_WO, T_END = 0, 8, 16, 24, 56, 64, 192, 200, 208

P2 = "e0 e1 w0 w1 w2 E0 p0 p1 p2 c E1 w3 w4 w5 E2 p3 p4 p5 c E3"
P4 = "e0 e1 w0 w1 w2 E0 p0 p1 p2 c E1 c w3 w4 w5 E2 p3 p4 p5 c E3 c"
PI = "e0 e1 w0 E0 p0 w1 p1 w2 E1 p2 w3 E2 p3 w4 p4 w5 E3 p5"
PO = "e0 e1 w0 E0 p0 c E1 w1 p1 w2 p2 c w3 E2 p3 c w4 p4 c E3 w5 p5 c"
PA = "w0 E0 p0 e0 c w1 p1 w2 E1 p2 w3 E2 p3 e1 c w4 p4 w5 E3 p5"
PB = "w0 E0 e0 c w1 w2 E1 p0 p1 p2 w3 E2 e1 c w4 w5 E3 p3 p4 p5"
PC = "w0 E0 e0 p0 p1 p2 c w1 w2 E1 w3 E2 e1 p3 p4 p5 c w4 w5 E3"
PD = "w0 E0 e0 p0 c w1 w2 E1 p1 p2 w3 E2 e1 p3 c w4 w5 E3 p4 p5"
PE = "w0 p0 w1 E0 e0 p1 c w2 w3 E1 p2 p3 w4 E2 e1 p4 c w5 p5 E3"
PF = "w0 E0 p0 w1 E1 e0 p1 c w2 w3 E2 p2 p3 w4 E3 e1 p4 c w5 p5"
PG = "w0 E0 e0 p0 p1 p2 c w1 E1 w2 w3 E2 e1 p3 p4 p5 c w4 E3 w5"
PO = "e0 e1 c c w0 w1 c w2 w3 c w4 w5 c"
PH = "w0 E0 e0 c p0 p1 p2 w1 E1 w2 w3 E2 e1 c p3 p4 p5 w4 E3 w5"


def build(L=3, L0=3, rot=16, compute=True, fs=(0, 4, 7, 3, 6, 2, 2, 6, 2, 6), ks=(0, 0, -2, -2, -4, -4, -5, -5, -5, -5),
          ls=(0, 4, 0, 4, 0, 4, 0, 4, 0, 4), M=33, bc=False, only=None, flags=None, plans={}, P=PH, pitch=24, scopes=False):
    fs, ks = [tuple(v + (L - L0) * (j >= 6) for j, v in enumerate(t)) for t in (fs, ks)]
    pn = dict(idle=PI, q=P, bq=P, ab=P, lat=P, ctx=P, kv=P, o0=P, out=P, o2=P, o1=PO)
    pn.update(plans)
    if not compute:
        pn = {k: pn["idle"] for k in pn}

    def kern(xa_h, k_h, v_h, wq_h, wo_h, xb_h, c_h, bwq_h, wuk_h, wuv_h, bwo_h, o_ref,
             xa_v, xb_v, k_v, v_v, wq_v, wo_v, c_v, bwq_v, wuk_v, wuv_v, bwo_v,
             qa_s, qb_s, qabs_s, sb_s, cc_s, oa_s, ob_s, lo_sem, hi_sem, x_sem):

        class Stream:
            def __init__(self, first, last, refs, rows, rot, place, steps):
                self.first, self.last, self.refs, self.rows, self.rot = first, last, refs, rows, rot
                self.place, self.steps = place, steps

            def copy(self, x, j, off, size, sem, wrap=False):
                src, dst = self.refs[j & 1]
                u = self.rows // 16
                so, do = self.place(x - self.first, self.steps[j], j & 1, self.rows, off * u // 16, wrap)
                n = size * u // 16
                dst = dst.at[pl.ds(pl.multiple_of(do, u), n)]
                if dst.shape[1:] != src.shape[1:]:
                    dst = dst.at[:, pl.ds(0, src.shape[1])]
                return pltpu.make_async_copy(src.at[pl.ds(pl.multiple_of(so, u), n)], dst, sem)

            def page(self, x, j):
                return self.copy(x, j, self.rot + 32 + 64 * (j >> 1), 64, lo_sem.at[(x & (RING - 1)) * 6 + j])

            def edge(self, x, j):
                off, sem = self.rot + 224 * (j >> 1), hi_sem.at[(x & (RING - 1)) * 2 + (j >> 1)]
                if self.rot and j == 3:
                    return [self.copy(x, 6 + j, off, 256 - off, sem),
                            self.copy(x, 6 + j, 256, off + 32 - 256, sem, True)]
                return [self.copy(x, 6 + j, off, 32, sem)]

        def flat(t, step, side, rows, off, wrap):
            o = ((t + step + wrap) & 7) * (2 * rows) + (0 if wrap else side * rows + off)
            return o, o

        def flat_c(t, step, side, rows, off, wrap):
            o = (((t + step + wrap) & 7) + (t & -8)) * (2 * rows) + (0 if wrap else side * rows + off)
            return o, o

        def window(t, step, side, rows, off, wrap):
            h = (t * M + step * M) & 127
            return h * (4 * rows) + (3 * rows + off), h * rows + off

        def both(src, dst):
            return ((src, dst), (src, dst))

        st_wq = Stream(T_WQ, T_BWQ, both(wq_h, wq_v), 128, 0, flat, fs)
        st_kv = Stream(T_KV, T_BWO, ((k_h.bitcast(U32), k_v), (v_h.bitcast(U32), v_v)), 512, 0, window, ks)
        streams = [
            st_wq,
            Stream(T_BWQ, T_WUK, both(bwq_h.bitcast(U32), bwq_v), 32, rot, flat, fs),
            Stream(T_WUK, T_C, both(wuk_h.bitcast(U32), wuk_v), 32, rot, flat, fs),
            Stream(T_C, T_WUV, both(c_h, c_v), 256, rot, flat_c, fs),
            Stream(T_WUV, T_KV, both(wuv_h.bitcast(U32), wuv_v), 32, rot, flat, fs),
            st_kv,
            Stream(T_BWO, T_WO, both(bwo_h, bwo_v), 256, rot, flat, fs),
            Stream(T_WO, T_END, both(wo_h, wo_v), 256, 0, flat, ls),
        ]

        def owner(x):
            return next((st for st in streams if st.first <= x < st.last), None)

        def start_edge(st, x, j):
            for cp in st.edge(x, j):
                cp.start()

        def run(lo, hi, name, body=None, carry=0):
            def it(sp, se, g, carry):
                on = body is not None and compute and (only is None or name in only)
                segs = body(g, carry) if on else iter(())
                for op in pn[name].split():
                    if op[0] == "e":
                        whole = k_v.at[pl.ds(0, 128)]
                        pltpu.make_async_copy(whole, whole, hi_sem.at[(g & (RING - 1)) * 2 + int(op[1])]).wait()
                    elif op == "c":
                        carry = next(segs, carry)
                    elif op[0] == "w":
                        st_kv.page(g, int(op[1])).wait()
                    elif op[0] == "p" and sp:
                        sp.page(g + L, int(op[1])).start(priority=1)
                    elif op[0] == "E" and se:
                        start_edge(se, g + L0, int(op[1]))
                for carry in segs:
                    pass
                return carry
            cuts = sorted({lo, hi} | {st.last - k for st in streams for k in (L, L0) if lo < st.last - k < hi})
            with jax.named_scope("ph_" + name) if scopes else contextlib.nullcontext():
                for a, b in zip(cuts, cuts[1:]):
                    step = functools.partial(it, owner(a + L), owner(a + L0))
                    carry = step(a, carry) if b == a + 1 else lax.fori_loop(a, b, step, carry)
            return carry

        def first(x, c):
            for j in range(6):
                st_wq.page(x, j).start(priority=1)

            @pl.when(x < L0)
            def _():
                for j in range(4):
                    start_edge(st_wq, x, j)
            return c
        lax.fori_loop(0, L, first, 0)
        xcp = [pltpu.make_async_copy(xa_h, xa_v, x_sem.at[0]), pltpu.make_async_copy(xb_h, xb_v, x_sem.at[1])]
        for cp in xcp:
            cp.start(priority=1)
        run(0, T_BWQ, "idle")
        for cp in xcp:
            cp.wait()

        def split(name, i):
            return pn[name].count("c") == 4 or i & 1

        def q_body(g, c):
            for i in range(4):
                h = (g - T_BWQ) * 4 + i
                w = jnp.concatenate([wq_v[r * NH + h] for r in range(DM // 8)], axis=0)
                qa_s[pl.ds(h, NB, stride=NH), :] = jnp.dot(xa_v[...], w, preferred_element_type=F32)
                if split("q", i):
                    yield c
        run(T_BWQ, T_WUK, "q", q_body)

        def head_pairs(w_v, t):
            for i in range(2):
                w = w_v.reshape(DM * pitch, DH)[pl.ds(2 * t + i, DM, stride=pitch), :]
                yield 4 * t + 2 * i, pltpu.bitcast(w << 16, F32).astype(BF16)
                yield 4 * t + 2 * i + 1, pltpu.bitcast(w & jnp.uint32(0xFFFF0000), F32).astype(BF16)

        def bq_body(g, c):
            for i, (h, w) in enumerate(head_pairs(bwq_v, g - T_WUK)):
                qb_s[h] = jnp.dot(xb_v[...], w, preferred_element_type=F32)
                if split("bq", i):
                    yield c
        run(T_WUK, T_C, "bq", bq_body)

        def abs_body(g, c):
            for i, (h, w) in enumerate(head_pairs(wuk_v, g - T_C)):
                r = lax.dot_general(qb_s[h].astype(BF16), w, NT, preferred_element_type=F32)
                for t in range(4):
                    qabs_s[t, pl.ds(h, NB, stride=NH), :] = r[:, t * 128:(t + 1) * 128]
                if split("ab", i):
                    yield c
        run(T_C, T_C + 8, "ab", abs_body)

        def lat_keys(t):
            return c_v[pl.ds(pl.multiple_of(t * 512, 512), 512), :]

        def lat_scores(t):
            r0 = pl.multiple_of((t >> 3) * NH, NH)
            q = jnp.concatenate([qabs_s[i, pl.ds(r0, NH), :] for i in range(4)], axis=1).astype(BF16)
            sb_s[...] = lax.dot_general(q, lat_keys(t), NT, preferred_element_type=F32) * SCALE

        def lat_body(g, carry):
            m, l = carry
            t = g - (T_C + 8)
            r0 = pl.multiple_of((t >> 3) * NH, NH)
            fresh = (t & 7) == 0
            m = jnp.where(fresh, -jnp.inf, m)
            s0 = sb_s[...]
            m_new = jnp.maximum(m, jnp.max(s0, axis=1, keepdims=True))
            alpha = jnp.exp(m - m_new)
            p = jnp.exp(s0 - m_new)
            l = jnp.where(fresh, 0.0, alpha * l) + jnp.sum(p, axis=1, keepdims=True)
            p = p.astype(BF16)
            lat_scores(jnp.minimum(t + 1, 31))
            yield carry
            pv = jnp.dot(p, lat_keys(t), preferred_element_type=F32)
            norm = jnp.where((t & 7) == 7, 1.0 / l, 1.0)
            for i in range(4):
                acc = cc_s[i, pl.ds(r0, NH), :]
                cc_s[i, pl.ds(r0, NH), :] = (alpha * acc + pv[:, i * 128:(i + 1) * 128]) * norm
            yield m_new, l
        if compute:
            cc_s[...] = jnp.zeros(cc_s.shape, F32)
            lat_scores(0)
        run(T_C + 8, T_KV, "lat", lat_body, (jnp.zeros((NH, 1), F32), jnp.zeros((NH, 1), F32)))

        def ctx_body(g, c):
            for i, (h, w) in enumerate(head_pairs(wuv_v, g - T_KV)):
                cc = jnp.concatenate([cc_s[t, pl.ds(h, NB, stride=NH), :] for t in range(4)], axis=1)
                ob_s[h] = jnp.dot(cc.astype(BF16), w, preferred_element_type=F32)
                if split("ctx", i):
                    yield c
        run(T_KV, T_KV + 8, "ctx", ctx_body)

        def kv_rows(ref, h):
            return pltpu.bitcast(ref[pl.ds(pl.multiple_of(h * 512, 512), 512), :], BF16)

        def kv_scores(i):
            h = (i * M) & 127
            q = jnp.broadcast_to(qa_s[pl.ds(h, 1), :], (8, DH)).astype(BF16)
            return lax.dot_general(q, kv_rows(k_v, h), NT, preferred_element_type=F32) * SCALE

        def kv_body(g, s0):
            i = g - (T_KV + 8)
            h = (i * M) & 127
            p = jnp.exp(s0 - jnp.max(s0, axis=1, keepdims=True))
            norm = 1.0 / jnp.sum(p, axis=1, keepdims=True)
            p = p.astype(BF16)
            s1 = kv_scores(jnp.minimum(i + 1, 127))
            yield s0
            o = jnp.dot(p, kv_rows(v_v, h), preferred_element_type=F32) * norm
            oa_s[pl.ds(h, 1), :] = o[0:1]
            t = i & 31
            yield s1
        run(T_KV + 8, T_WO, "kv", kv_body, kv_scores(0) if compute else 0)

        def project(o, w_v, h):
            return jnp.dot(o.astype(BF16), w_v[pl.ds(pl.multiple_of(h * DH, DH), DH), :], preferred_element_type=F32)

        def a_proj(t, i):
            h = ((t + 4 * (i & 1)) & 7) * 4 + 2 * (i & 1) + (i >> 1)
            return project(oa_s[pl.ds(h, NB, stride=NH), :], wo_v, h)

        def b_proj(yb, h0, n):
            for i in range(n):
                yb = yb + project(ob_s[h0 + i], bwo_v, h0 + i)
            return yb

        def out_first(g, yb):
            yb = b_proj(yb, 0, 4)
            yield yb
            yield b_proj(yb, 4, 4)

        def out_body(g, carry):
            ya, yb = carry
            t = g - (T_WO + 1)
            for i in range(4):
                ya = ya + a_proj(t, i)
            yield ya, yb
            yield ya, b_proj(yb, 8 + 6 * t, 6)

        def out_tail(g, ya):
            t = g - (T_WO + 1)
            for i in range(4):
                ya = ya + a_proj(t, i)
                if i & 1:
                    yield ya

        def out_last(g, ya):
            for i in range(4):
                ya = ya + a_proj(6, i)
            heads = [28, 14]
            o = [jnp.concatenate([oa_s[pl.ds(h + i, NB, stride=NH), :] for i in range(2)], axis=1) for h in heads]
            groups = [[(0, 32), (224, 32)], [(32, 64)], [(96, 64)], [(160, 64)]]
            lhs = [jnp.concatenate([o[s][:, r:r + n] for s in range(2) for r, n in grp], axis=1).astype(BF16)
                   for grp in groups]
            yield ya
            for x, grp in zip(lhs, groups):
                w = jnp.concatenate([wo_v[pl.ds(h * DH + r, n), :] for h in heads for r, n in grp], axis=0)
                ya = ya + jnp.dot(x, w, preferred_element_type=F32)
                yield ya

        z = jnp.zeros((NB, DM), F32)
        yb = run(T_WO, T_WO + 1, "o0", out_first, z)
        ya, yb = run(T_WO + 1, T_WO + 5, "out", out_body, (z, yb))
        o_ref[:, DM:2 * DM] = yb.astype(BF16)
        ya = run(T_WO + 5, T_END - 1, "o2", out_tail, ya)
        ya = run(T_END - 1, T_END, "o1", out_last, ya)
        o_ref[:, 0:DM] = ya.astype(BF16)

    @jax.jit
    def f(A_x, A_k_cache, A_v_cache, A_wq, A_wo, B_x, B_c_kv, B_w_q, B_w_uk, B_w_uv, B_w_o):
        vm = pltpu.VMEM
        wq = A_wq.reshape(DM // 8, 8, NH, DH).transpose(0, 2, 1, 3).reshape(DM // 8 * NH, 8, DH)
        out = pl.pallas_call(
            kern,
            out_shape=jax.ShapeDtypeStruct((NB, 2 * DM), BF16),
            in_specs=[pl.BlockSpec(memory_space=pl.ANY)] * 11,
            out_specs=pl.BlockSpec(memory_space=vm),
            scratch_shapes=[
                vm((NB, DM), BF16), vm((NB, DM), BF16),
                vm((NB * NH * WIN // 2, DH), U32), vm((NB * NH * WIN // 2, DH), U32),
                vm((DM // 8 * NH, 8, DH), BF16), vm((NH * DH, DM), BF16), vm((NB * SK, DM), BF16),
                vm((DM, pitch, DH), U32), vm((DM, pitch, DH), U32), vm((DM, pitch, DH), U32),
                vm((NH * DH, DM), BF16),
                vm((NB * NH, DH), F32), vm((NH, NB, DH), F32), vm((4, NB * NH, 128), F32),
                vm((NH, 512), F32), vm((4, NB * NH, 128), F32), vm((NB * NH, DH), F32), vm((NH, NB, DH), F32),
                pltpu.SemaphoreType.DMA((RING * 6,)), pltpu.SemaphoreType.DMA((RING * 2,)), pltpu.SemaphoreType.DMA((2,)),
            ],
            compiler_params=pltpu.CompilerParams(vmem_limit_bytes=120 * 1024 * 1024, disable_bounds_checks=not bc, disable_semaphore_checks=True, flags=flags),
        )(A_x.reshape(NB, DM), A_k_cache.reshape(-1, DH), A_v_cache.reshape(-1, DH), wq, A_wo,
          B_x.reshape(NB, DM), B_c_kv.reshape(-1, DM), B_w_q, B_w_uk,
          B_w_uv, B_w_o.reshape(-1, DM))
        return out.reshape(NB, 1, 2 * DM)
    return f


pallas_concat_heads__sliding_block_cached__compressed_kv_cla__decode_kernel = build()
```

```python
import contextlib
import functools
import jax
import jax.numpy as jnp
from jax import lax
from jax.experimental import pallas as pl
from jax.experimental.pallas import tpu as pltpu

NB, NH, DH, DM, SK = 4, 32, 128, 512, 4096
WIN = 1024
F32, BF16, U32 = jnp.float32, jnp.bfloat16, jnp.uint32
NT = (((1,), (1,)), ((), ()))
RING = 4
SCALE = DH ** -0.5
T_WQ, T_BWQ, T_WUK, T_C, T_WUV, T_KV, T_BWO, T_WO, T_END = 0, 8, 16, 24, 56, 64, 192, 200, 208

PH = "w0 E0 e0 c p0 p1 p2 w1 E1 w2 w3 E2 e1 c p3 p4 p5 w4 E3 w5"
PL2 = "w0 E0 e0 c E1 c p0 p1 p2 w1 w2 w3 E2 e1 c p3 p4 p5 w4 E3 w5"
PO = "c w0 w1 e0 e1 c c w2 w3 c w4 w5 c"

FLAT4 = ([[(j, 0, 64)] for j in range(6)], [(7, 0, 32), (7, 32, 32), (6, 0, 32), (6, 32, 32)])
FLAT6 = ([[(0, 0, 64)], [(1, 0, 64)], [(2, 0, 64)], [(3, 0, 32)], [(3, 32, 32)], [(4, 0, 64)]],
         [(5 + i // 2, 32 * (i & 1), 32) for i in range(6)])
KV4 = ([[((j & 1, -2 * (j >> 1)), 32 + 64 * (j >> 1), 64)] for j in range(6)],
       [((j & 1, -5), 224 * (j >> 1), 32) for j in range(4)])
KV6 = ([[((0, 0), 32, 64)], [((1, 0), 32, 64)], [((1, -2), 96, 64)], [((0, -4), 160, 32)], [((0, -4), 192, 32)],
        [((1, -4), 160, 64)]],
       [((1, -5), 0, 32), ((0, -6), 96, 32), ((0, -6), 128, 32), ((0, -5), 0, 32), ((1, -5), 224, 32), ((0, -5), 224, 32)])
LAST = ([[((j & 1, 4 * (j & 1)), 32 + 64 * (j >> 1), 64)] for j in range(6)],
        [((j & 1, 4 * (j & 1)), 224 * (j >> 1), 32) for j in range(4)])


def build(L=3, sa=32, sb=48, M=33, only=None, flags=None, plans={}, P=PH, pitch=24, scopes=False, pre=2,
          tail=(4, 3, 3, 3, 3, 0), pat={}, ksplit=512, manual=0):
    pn = dict(q=P, bq=P, ab=P, lat=PL2, ctx=P, kv=P, o0=P, out=P, o2=P, o1=PO)
    pn.update(plans)
    pt = dict(wq=FLAT4, bwq=FLAT4, wuk=FLAT4, c=FLAT4, wuv=FLAT4, kv=KV4, bwo=FLAT4, wo=LAST)
    pt.update(pat)

    def kern(xa_h, k_h, v_h, wq_h, wo_h, xb_h, c_h, bwq_h, wuk_h, wuv_h, bwo_h, o_ref,
             xa_v, xb_v, k_v, v_v, wq_v, wo_v, c_v, bwq_v, wuk_v, wuv_v, bwo_v,
             qa_s, qb_s, qabs_s, sb_s, cc_s, oa_s, ob_s, o_v, lo_sem, hi_sem, x_sem):

        def dma(src, dst, rows, so, do, size, sem):
            u = rows // 16
            n = size * u // 16
            dst = dst.at[pl.ds(pl.multiple_of(do, u), n)]
            if dst.shape[1:] != src.shape[1:]:
                dst = dst.at[:, pl.ds(0, src.shape[1])]
            return pltpu.make_async_copy(src.at[pl.ds(pl.multiple_of(so, u), n)], dst, sem)

        def flat(src, dst, rows, shift, batched=False):
            def copies(t, piece, sem):
                region, off, size = piece
                o = region * 512 + shift + off
                base = (t & -8) * (2 * rows) if batched else 0

                def one(o, size):
                    r = (t & 7) * (rows // 4) + o * rows // 256
                    if o + 7 * 64 >= 4096:
                        r = r & (16 * rows - 1)
                    return dma(src, dst, rows, base + r, base + r, size, sem)
                cut = 4096 - 7 * 64 - o
                if 0 < cut < size:
                    return [one(o, cut), one(o + cut, size - cut)]
                return [one(o, size)]
            return copies

        def window(t, piece, sem):
            (side, lag), off, size = piece
            src, dst = ((k_h, k_v), (v_h, v_v))[side]
            h = (t * M + lag * M) & 127
            return [dma(src.bitcast(U32), dst, 512, h * 2048 + (1536 + 2 * off), h * 512 + 2 * off, size, sem)]

        def last(t, piece, sem):
            (side, lag), off, size = piece
            r = ((t + lag) & 7) * 512 + (side * 256 + off)
            return [dma(wo_h, wo_v, 256, r, r, size, sem)]

        streams = [
            (T_WQ, T_BWQ, flat(wq_h, wq_v, 128, sa), pt["wq"]),
            (T_BWQ, T_WUK, flat(bwq_h.bitcast(U32), bwq_v, 32, sb), pt["bwq"]),
            (T_WUK, T_C, flat(wuk_h.bitcast(U32), wuk_v, 32, sb), pt["wuk"]),
            (T_C, T_WUV, flat(c_h, c_v, 256, sb, True), pt["c"]),
            (T_WUV, T_KV, flat(wuv_h.bitcast(U32), wuv_v, 32, sb), pt["wuv"]),
            (T_KV, T_BWO, window, pt["kv"]),
            (T_BWO, T_WO, flat(bwo_h, bwo_v, 256, sb), pt["bwo"]),
            (T_WO, T_END, last, pt["wo"]),
        ]

        def owner(x):
            return next((st for st in streams if st[0] <= x < st[1]), None)

        def low(st, x, j):
            return [cp for piece in st[3][0][j] for cp in st[2](x - st[0], piece, lo_sem.at[(x & (RING - 1)) * 6 + j])]

        def high(st, x, j, sem=None):
            half = j * 2 // len(st[3][1])
            return st[2](x - st[0], st[3][1][j], hi_sem.at[(x & (RING - 1)) * 2 + half] if sem is None else sem)

        def start(copies, prio):
            for cp in copies:
                cp.start(priority=prio)

        late = [(x, j) for x in range(T_END - 4, T_END) for j in range(4)]

        def run(lo, hi, name, body=None, carry=0):
            def it(sw, sp, g, carry):
                on = only is None or name in only
                segs = body(g, carry) if on else iter(())
                for op in pn[name].split():
                    if op[0] == "e":
                        n = len(sw[3][1]) // 2
                        for j in range(n):
                            for cp in high(sw, g, int(op[1]) * n + j):
                                cp.wait()
                    elif op == "c":
                        carry = next(segs, carry)
                    elif op[0] == "w":
                        for cp in low(sw, g, int(op[1])):
                            cp.wait()
                    elif op[0] == "p" and sp:
                        start(low(sp, g + L, int(op[1])), 1)
                    elif op[0] == "E" and tail and isinstance(g, int) and g > T_WO:
                        k = tail[g - T_WO - 1]
                        if int(op[1]) in ((), (0,), (0, 2), (0, 1, 3), (0, 1, 2, 3))[k]:
                            start(high(streams[-1], *late.pop(0)), 0)
                    elif op[0] in "EF" and sp:
                        n = len(sp[3][1])
                        j = {("E", 4): (0, 1, 2, 3), ("E", 6): (0, 2, 3, 5), ("F", 4): (), ("F", 6): (1, 4)}[op[0], n]
                        if j:
                            start(high(sp, g + L, j[int(op[1])]), 0)
                for carry in segs:
                    pass
                return carry
            cuts = sorted({lo, hi} | {st[1] - k for st in streams for k in (0, L) if lo < st[1] - k < hi})
            if tail and lo >= T_WO:
                cuts = list(range(lo, hi + 1))
            with jax.named_scope("ph_" + name) if scopes else contextlib.nullcontext():
                for a, b in zip(cuts, cuts[1:]):
                    step = functools.partial(it, owner(a), owner(a + L))
                    carry = step(a, carry) if b == a + 1 else lax.fori_loop(a, b, step, carry)
            return carry

        xcp = [pltpu.make_async_copy(xa_h, xa_v, x_sem.at[0]), pltpu.make_async_copy(xb_h, xb_v, x_sem.at[1])]
        todo = [high(owner(x), x, j, x_sem.at[2] if x < T_BWQ else None)
                for x in range(T_BWQ + L) for j in range(len(owner(x)[3][1]))]
        first = sum(todo[:T_BWQ * len(pt["wq"][1])], [])
        npre = max(pre, len(todo) - 6 * T_BWQ)
        for x in range(L):
            for j in range(6):
                start(low(streams[0], x, j), 1)
                i = x * 6 + j
                for _ in range((i + 1) * npre // (6 * L) - i * npre // (6 * L)):
                    start(todo.pop(0), 0)
        start(xcp, 1)
        for g in range(T_BWQ):
            for j in range(6):
                for cp in low(streams[0], g, j):
                    cp.wait()
                if todo:
                    start(todo.pop(0), 0)
                start(low(owner(g + L), g + L, j), 1)
        with jax.named_scope('ph_idle') if scopes else contextlib.nullcontext():
            for cp in first + xcp:
                cp.wait()

        def q_body(g, c):
            for i in range(4):
                h = (g - T_BWQ) * 4 + i
                w = jnp.concatenate([wq_v[r * NH + h] for r in range(DM // 8)], axis=0)
                qa_s[pl.ds(h, NB, stride=NH), :] = jnp.dot(xa_v[...], w, preferred_element_type=F32)
                if i & 1:
                    yield c
        run(T_BWQ, T_WUK, "q", q_body)

        def head_pairs(w_v, t):
            for i in range(2):
                w = w_v.reshape(DM * pitch, DH)[pl.ds(2 * t + i, DM, stride=pitch), :]
                yield 4 * t + 2 * i, pltpu.bitcast(w << 16, F32).astype(BF16)
                yield 4 * t + 2 * i + 1, pltpu.bitcast(w & jnp.uint32(0xFFFF0000), F32).astype(BF16)

        def bq_body(g, c):
            for i, (h, w) in enumerate(head_pairs(bwq_v, g - T_WUK)):
                qb_s[h] = jnp.dot(xb_v[...], w, preferred_element_type=F32)
                if i & 1:
                    yield c
        run(T_WUK, T_C, "bq", bq_body)

        def abs_body(g, c):
            for i, (h, w) in enumerate(head_pairs(wuk_v, g - T_C)):
                r = lax.dot_general(qb_s[h].astype(BF16), w, NT, preferred_element_type=F32)
                for t in range(4):
                    qabs_s[t, pl.ds(h, NB, stride=NH), :] = r[:, t * 128:(t + 1) * 128]
                if i & 1:
                    yield c
        run(T_C, T_C + 8, "ab", abs_body)

        def lat_scores(t):
            r0 = pl.multiple_of((t >> 3) * NH, NH)
            q = jnp.concatenate([qabs_s[i, pl.ds(r0, NH), :] for i in range(4)], axis=1).astype(BF16)
            for i in range(2):
                keys = c_v[pl.ds(pl.multiple_of(t * 512 + i * 256, 256), 256), :]
                sb_s[:, i * 256:(i + 1) * 256] = lax.dot_general(q, keys, NT, preferred_element_type=F32) * SCALE
                yield

        def lat_body(g, carry):
            m, l = carry
            t = g - (T_C + 8)
            r0 = pl.multiple_of((t >> 3) * NH, NH)
            fresh = (t & 7) == 0
            m = jnp.where(fresh, -jnp.inf, m)
            s0 = sb_s[...]
            m_new = jnp.maximum(m, jnp.max(s0, axis=1, keepdims=True))
            alpha = jnp.exp(m - m_new)
            p = jnp.exp(s0 - m_new)
            l = jnp.where(fresh, 0.0, alpha * l) + jnp.sum(p, axis=1, keepdims=True)
            p = p.astype(BF16)
            for _ in lat_scores(jnp.minimum(t + 1, 31)):
                yield carry
            n = pn["lat"].split().count("c") - 2
            pv = 0
            for i in range(n):
                keys = c_v[pl.ds(pl.multiple_of(t * 512 + i * (512 // n), 256), 512 // n), :]
                pv = pv + jnp.dot(p[:, i * (512 // n):(i + 1) * (512 // n)], keys, preferred_element_type=F32)
                if i < n - 1:
                    yield carry
            norm = jnp.where((t & 7) == 7, 1.0 / l, 1.0)
            for i in range(4):
                acc = cc_s[i, pl.ds(r0, NH), :]
                cc_s[i, pl.ds(r0, NH), :] = (alpha * acc + pv[:, i * 128:(i + 1) * 128]) * norm
            yield m_new, l
        if only is None or "lat" in only:
            cc_s[...] = jnp.zeros(cc_s.shape, F32)
            list(lat_scores(0))
        run(T_C + 8, T_KV, "lat", lat_body, (jnp.zeros((NH, 1), F32), jnp.zeros((NH, 1), F32)))

        def ctx_body(g, c):
            for i, (h, w) in enumerate(head_pairs(wuv_v, g - T_KV)):
                cc = jnp.concatenate([cc_s[t, pl.ds(h, NB, stride=NH), :] for t in range(4)], axis=1)
                ob_s[h] = jnp.dot(cc.astype(BF16), w, preferred_element_type=F32)
                if i & 1:
                    yield c
        run(T_KV, T_KV + 8, "ctx", ctx_body)

        def kv_rows(ref, h, a, b):
            return pltpu.bitcast(ref[pl.ds(pl.multiple_of(h * 512 + a // 2, 64), (b - a) // 2), :], BF16)

        def kv_scores(i, a, b):
            h = (i * M) & 127
            q = jnp.broadcast_to(qa_s[pl.ds(h, 1), :], (8, DH)).astype(BF16)
            return lax.dot_general(q, kv_rows(k_v, h, a, b), NT, preferred_element_type=F32) * SCALE

        def kv_body(g, s0):
            i = g - (T_KV + 8)
            h = (i * M) & 127
            p = jnp.exp(s0 - jnp.max(s0, axis=1, keepdims=True))
            norm = 1.0 / jnp.sum(p, axis=1, keepdims=True)
            p = p.astype(BF16)
            parts = [(0, WIN)] if pn["kv"].split().count("c") == 2 else [(0, ksplit), (ksplit, WIN)]
            s1 = []
            for a, b in parts:
                s1.append(kv_scores(jnp.minimum(i + 1, 127), a, b))
                yield s0
            o = 0
            for a, b in parts:
                o = o + jnp.dot(p[:, a:b], kv_rows(v_v, h, a, b), preferred_element_type=F32)
                if b < WIN:
                    yield s0
            oa_s[pl.ds(h, 1), :] = (o * norm)[0:1]
            yield jnp.concatenate(s1, axis=1)
        run(T_KV + 8, T_WO, "kv", kv_body, kv_scores(0, 0, WIN) if only is None or "kv" in only else 0)

        def project(o, w_v, h):
            return jnp.dot(o.astype(BF16), w_v[pl.ds(pl.multiple_of(h * DH, DH), DH), :], preferred_element_type=F32)

        def a_proj(t, i):
            h = ((t + 4 * (i & 1)) & 7) * 4 + 2 * (i & 1) + (i >> 1)
            return project(oa_s[pl.ds(h, NB, stride=NH), :], wo_v, h)

        def b_proj(yb, h0, n):
            for i in range(n):
                yb = yb + project(ob_s[h0 + i], bwo_v, h0 + i)
            return yb

        def out_first(g, yb):
            yb = b_proj(yb, 0, 4)
            yield yb
            yield b_proj(yb, 4, 4)

        def out_body(g, carry):
            ya, yb = carry
            t = g - (T_WO + 1)
            for i in range(4):
                ya = ya + a_proj(t, i)
            yield ya, yb
            yield ya, b_proj(yb, 8 + 6 * t, 6)

        def out_tail(g, ya):
            t = g - (T_WO + 1)
            for i in range(4):
                ya = ya + a_proj(t, i)
                if i & 1:
                    yield ya

        def out_last(g, ya):
            for i in range(4):
                ya = ya + a_proj(6, i)
            heads = [28, 14]
            o = [jnp.concatenate([oa_s[pl.ds(h + i, NB, stride=NH), :] for i in range(2)], axis=1) for h in heads]
            groups = [[(32, 64)], [(0, 32), (224, 32)], [(96, 64)], [(160, 64)]]
            lhs = [jnp.concatenate([o[s][:, r:r + n] for s in range(2) for r, n in grp], axis=1).astype(BF16)
                   for grp in groups]
            yield ya
            for x, grp in zip(lhs, groups):
                w = jnp.concatenate([wo_v[pl.ds(h * DH + r, n), :] for h in heads for r, n in grp], axis=0)
                ya = ya + jnp.dot(x, w, preferred_element_type=F32)
                yield ya

        z = jnp.zeros((NB, DM), F32)
        yb = run(T_WO, T_WO + 1, "o0", out_first, z)
        ya, yb = run(T_WO + 1, T_WO + 5, "out", out_body, (z, yb))
        dst = o_v if manual else o_ref
        dst[:, DM:2 * DM] = yb.astype(BF16)
        if manual == 2:
            cb = pltpu.make_async_copy(o_v.at[:, DM:2 * DM], o_ref.at[:, DM:2 * DM], x_sem.at[1])
            cb.start()
        ya = run(T_WO + 5, T_END - 1, "o2", out_tail, ya)
        ya = run(T_END - 1, T_END, "o1", out_last, ya)
        dst[:, 0:DM] = ya.astype(BF16)
        if manual:
            w = DM if manual == 2 else 2 * DM
            ca = pltpu.make_async_copy(o_v.at[:, 0:w], o_ref.at[:, 0:w], x_sem.at[0])
            ca.start()
            if manual == 2:
                cb.wait()
            ca.wait()

    @jax.jit
    def f(A_x, A_k_cache, A_v_cache, A_wq, A_wo, B_x, B_c_kv, B_w_q, B_w_uk, B_w_uv, B_w_o):
        vm = pltpu.VMEM
        wq = A_wq.reshape(DM // 8, 8, NH, DH).transpose(0, 2, 1, 3).reshape(DM // 8 * NH, 8, DH)
        out = pl.pallas_call(
            kern,
            out_shape=jax.ShapeDtypeStruct((NB, 2 * DM), BF16),
            in_specs=[pl.BlockSpec(memory_space=pl.ANY)] * 11,
            out_specs=pl.BlockSpec(memory_space=pl.ANY if manual else vm),
            scratch_shapes=[
                vm((NB, DM), BF16), vm((NB, DM), BF16),
                vm((NB * NH * WIN // 2, DH), U32), vm((NB * NH * WIN // 2, DH), U32),
                vm((DM // 8 * NH, 8, DH), BF16), vm((NH * DH, DM), BF16), vm((NB * SK, DM), BF16),
                vm((DM, pitch, DH), U32), vm((DM, pitch, DH), U32), vm((DM, pitch, DH), U32),
                vm((NH * DH, DM), BF16),
                vm((NB * NH, DH), F32), vm((NH, NB, DH), F32), vm((4, NB * NH, 128), F32),
                vm((NH, 512), F32), vm((4, NB * NH, 128), F32), vm((NB * NH, DH), F32), vm((NH, NB, DH), F32),
                vm((NB, 2 * DM), BF16),
                pltpu.SemaphoreType.DMA((RING * 6,)), pltpu.SemaphoreType.DMA((RING * 2,)), pltpu.SemaphoreType.DMA((3,)),
            ],
            compiler_params=pltpu.CompilerParams(vmem_limit_bytes=120 * 1024 * 1024, disable_bounds_checks=True,
                                                 disable_semaphore_checks=True, flags=flags),
        )(A_x.reshape(NB, DM), A_k_cache.reshape(-1, DH), A_v_cache.reshape(-1, DH), wq, A_wo,
          B_x.reshape(NB, DM), B_c_kv.reshape(-1, DM), B_w_q, B_w_uk, B_w_uv, B_w_o.reshape(-1, DM))
        return out.reshape(NB, 1, 2 * DM)
    return f


pallas_concat_heads__sliding_block_cached__compressed_kv_cla__decode_kernel = build()
```

```python
import contextlib
import functools
import jax
import jax.numpy as jnp
from jax import lax
from jax.experimental import pallas as pl
from jax.experimental.pallas import tpu as pltpu

NB, NH, DH, DM, SK = 4, 32, 128, 512, 4096
WIN = 1024
F32, BF16, U32 = jnp.float32, jnp.bfloat16, jnp.uint32
NT = (((1,), (1,)), ((), ()))
RING = 4
SCALE = DH ** -0.5
T_WQ, T_BWQ, T_WUK, T_C, T_WUV, T_KV, T_BWO, T_WO, T_END = 0, 8, 16, 24, 56, 64, 192, 200, 208

PH = "w0 E0 e0 c p0 p1 p2 w1 E1 w2 w3 E2 e1 c p3 p4 p5 w4 E3 w5"
PL2 = "w0 E0 e0 c E1 c p0 p1 p2 w1 w2 w3 E2 e1 c p3 p4 p5 w4 E3 w5"
PO = "c w0 w1 e0 e1 c c w2 w3 c w4 w5 c"

FLAT4 = ([[(j, 0, 64)] for j in range(6)], [(7, 0, 32), (7, 32, 32), (6, 0, 32), (6, 32, 32)])
FLAT6 = ([[(0, 0, 64)], [(1, 0, 64)], [(2, 0, 64)], [(3, 0, 32)], [(3, 32, 32)], [(4, 0, 64)]],
         [(5 + i // 2, 32 * (i & 1), 32) for i in range(6)])
KV4 = ([[((j & 1, -2 * (j >> 1)), 32 + 64 * (j >> 1), 64)] for j in range(6)],
       [((j & 1, -5), 224 * (j >> 1), 32) for j in range(4)])
KV6 = ([[((0, 0), 32, 64)], [((1, 0), 32, 64)], [((1, -2), 96, 64)], [((0, -4), 160, 32)], [((0, -4), 192, 32)],
        [((1, -4), 160, 64)]],
       [((1, -5), 0, 32), ((0, -6), 96, 32), ((0, -6), 128, 32), ((0, -5), 0, 32), ((1, -5), 224, 32), ((0, -5), 224, 32)])
LAST = ([[((j & 1, 4 * (j & 1)), 32 + 64 * (j >> 1), 64)] for j in range(6)],
        [((j & 1, 4 * (j & 1)), 224 * (j >> 1), 32) for j in range(4)])
K6A = "w0 H0 e0 c H1 c p0 p1 p2 w1 H2 w2 w3 H3 e1 c p3 p4 p5 w4 H4 w5 H5"
K6B = "w0 H0 e0 c H1 c p0 p1 p2 w1 w2 H2 w3 H3 e1 c p3 p4 p5 w4 H4 w5 H5"
K6C = "w0 H0 e0 c w1 H1 e1 c p0 p1 p2 w2 H2 w3 H3 w4 H4 c p3 p4 p5 w5 H5"
K6D = "w0 H0 e0 c w1 H1 e1 c p0 p1 p2 w2 H2 w3 c H3 c p3 p4 p5 w4 H4 w5 H5"
KV6 = (KV6[0], [KV6[1][i] for i in (3, 1, 2, 0, 4, 5)])
KV5 = (KV4[0], KV4[1][:3] + [((1, -5), 224, 16), ((1, -5), 240, 16)])
KV6 = (KV4[0], [((0, -5), 0, 32), ((1, -5), 0, 16), ((1, -5), 16, 16)] + KV5[1][2:])
FLAT5 = (FLAT4[0], FLAT4[1][:3] + [(6, 32, 16), (6, 48, 16)])
FLAT6 = (FLAT4[0], [(7, 0, 32), (7, 32, 16), (7, 48, 16)] + FLAT5[1][2:])
P5 = "w0 E0 e0 c p0 p1 p2 w1 E1 w2 w3 E2 e1 c p3 p4 p5 w4 E3 w5 E4"
P6 = "w0 E0 e0 c p0 p1 p2 w1 E1 w2 F1 w3 E2 e1 c p3 p4 p5 w4 E3 w5 E4"
PL5 = "w0 E0 e0 c E1 c p0 p1 p2 w1 w2 w3 E2 e1 c p3 p4 p5 w4 E3 w5 E4"
PL6 = "w0 E0 e0 c E1 c p0 p1 p2 w1 F1 w2 w3 E2 e1 c p3 p4 p5 w4 E3 w5 E4"
ALL5 = dict(wq=FLAT5, bwq=FLAT5, wuk=FLAT5, c=FLAT5, wuv=FLAT5, kv=KV5, bwo=FLAT5)
ALL6 = dict(wq=FLAT6, bwq=FLAT6, wuk=FLAT6, c=FLAT6, wuv=FLAT6, kv=KV6, bwo=FLAT6)


def build(L=3, sa=32, sb=48, M=33, only=None, flags=None, plans={}, P=P6, pitch=24, scopes=False, pre=2,
          tail=(4, 3, 3, 3, 3, 0), pat={}, ksplit=(WIN, WIN), manual=0):
    pn = dict(q=P, bq=P, ab=P, lat=PL6, ctx=P, kv=P, o0=P, out=P, o2=P, o1=PO)
    pn.update(plans)
    pt = dict(wq=FLAT4, bwq=FLAT4, wuk=FLAT4, c=FLAT4, wuv=FLAT4, kv=KV4, bwo=FLAT4, wo=LAST)
    pt.update(eval(pat) if isinstance(pat, str) else pat)

    def kern(xa_h, k_h, v_h, wq_h, wo_h, xb_h, c_h, bwq_h, wuk_h, wuv_h, bwo_h, o_ref,
             xa_v, xb_v, k_v, v_v, wq_v, wo_v, c_v, bwq_v, wuk_v, wuv_v, bwo_v,
             qa_s, qb_s, qabs_s, sb_s, cc_s, oa_s, ob_s, o_v, lo_sem, hi_sem, x_sem):

        def dma(src, dst, rows, so, do, size, sem):
            u = rows // 16
            n = size * u // 16
            dst = dst.at[pl.ds(pl.multiple_of(do, u), n)]
            if dst.shape[1:] != src.shape[1:]:
                dst = dst.at[:, pl.ds(0, src.shape[1])]
            return pltpu.make_async_copy(src.at[pl.ds(pl.multiple_of(so, u), n)], dst, sem)

        def flat(src, dst, rows, shift, batched=False):
            def copies(t, piece, sem):
                region, off, size = piece
                o = region * 512 + shift + off
                base = (t & -8) * (2 * rows) if batched else 0

                def one(o, size):
                    r = (t & 7) * (rows // 4) + o * rows // 256
                    if o + 7 * 64 >= 4096:
                        r = r & (16 * rows - 1)
                    return dma(src, dst, rows, base + r, base + r, size, sem)
                cut = 4096 - 7 * 64 - o
                if 0 < cut < size:
                    return [one(o, cut), one(o + cut, size - cut)]
                return [one(o, size)]
            return copies

        def window(t, piece, sem):
            (side, lag), off, size = piece
            src, dst = ((k_h, k_v), (v_h, v_v))[side]
            h = (t * M + lag * M) & 127
            return [dma(src.bitcast(U32), dst, 512, h * 2048 + (1536 + 2 * off), h * 512 + 2 * off, size, sem)]

        def last(t, piece, sem):
            (side, lag), off, size = piece
            r = ((t + lag) & 7) * 512 + (side * 256 + off)
            return [dma(wo_h, wo_v, 256, r, r, size, sem)]

        streams = [
            (T_WQ, T_BWQ, flat(wq_h, wq_v, 128, sa), pt["wq"]),
            (T_BWQ, T_WUK, flat(bwq_h.bitcast(U32), bwq_v, 32, sb), pt["bwq"]),
            (T_WUK, T_C, flat(wuk_h.bitcast(U32), wuk_v, 32, sb), pt["wuk"]),
            (T_C, T_WUV, flat(c_h, c_v, 256, sb, True), pt["c"]),
            (T_WUV, T_KV, flat(wuv_h.bitcast(U32), wuv_v, 32, sb), pt["wuv"]),
            (T_KV, T_BWO, window, pt["kv"]),
            (T_BWO, T_WO, flat(bwo_h, bwo_v, 256, sb), pt["bwo"]),
            (T_WO, T_END, last, pt["wo"]),
        ]

        def owner(x):
            return next((st for st in streams if st[0] <= x < st[1]), None)

        def low(st, x, j):
            return [cp for piece in st[3][0][j] for cp in st[2](x - st[0], piece, lo_sem.at[(x & (RING - 1)) * 6 + j])]

        def high(st, x, j, sem=None):
            half = int(j >= len(st[3][1]) // 2)
            return st[2](x - st[0], st[3][1][j], hi_sem.at[(x & (RING - 1)) * 2 + half] if sem is None else sem)

        def start(copies, prio):
            for cp in copies:
                cp.start(priority=prio)

        late = [(x, j) for x in range(T_END - 4, T_END) for j in range(4)]

        def run(lo, hi, name, body=None, carry=0):
            def it(sw, sp, g, carry):
                on = only is None or name in only
                segs = body(g, carry) if on else iter(())
                for op in (pn[name] if name + "6" not in pn or not sp or len(sp[3][1]) == 4 else pn[name + "6"]).split():
                    if op[0] == "e":
                        n = len(sw[3][1]) // 2
                        for j in (range(n) if op == "e0" else range(n, len(sw[3][1]))):
                            for cp in high(sw, g, j):
                                cp.wait()
                    elif op == "c":
                        carry = next(segs, carry)
                    elif op[0] == "w":
                        for cp in low(sw, g, int(op[1])):
                            cp.wait()
                    elif op[0] == "p" and sp:
                        start(low(sp, g + L, int(op[1])), 1)
                    elif op[0] == "E" and tail and isinstance(g, int) and g > T_WO:
                        k = tail[g - T_WO - 1]
                        if int(op[1]) in ((), (0,), (0, 2), (0, 1, 3), (0, 1, 2, 3))[k] and op[0] == "E" and late:
                            start(high(streams[-1], *late.pop(0)), 0)
                    elif op[0] in "EF" and sp:
                        names = {4: "E0 E1 E2 E3", 5: "E0 E1 E2 E3 E4", 6: "E0 E1 F1 E2 E3 E4"}[len(sp[3][1])].split()
                        if op in names:
                            start(high(sp, g + L, names.index(op)), 0)
                for carry in segs:
                    pass
                return carry
            cuts = sorted({lo, hi} | {st[1] - k for st in streams for k in (0, L) if lo < st[1] - k < hi})
            if tail and lo >= T_WO:
                cuts = list(range(lo, hi + 1))
            with jax.named_scope("ph_" + name) if scopes else contextlib.nullcontext():
                for a, b in zip(cuts, cuts[1:]):
                    step = functools.partial(it, owner(a), owner(a + L))
                    carry = step(a, carry) if b == a + 1 else lax.fori_loop(a, b, step, carry)
            return carry

        xcp = [pltpu.make_async_copy(xa_h, xa_v, x_sem.at[0]), pltpu.make_async_copy(xb_h, xb_v, x_sem.at[1])]
        todo = [high(owner(x), x, j, x_sem.at[2] if x < T_BWQ else None)
                for x in range(T_BWQ + L) for j in range(len(owner(x)[3][1]))]
        first = sum(todo[:T_BWQ * len(pt["wq"][1])], [])
        npre = max(pre, len(todo) - 6 * T_BWQ)
        for x in range(L):
            for j in range(6):
                start(low(streams[0], x, j), 1)
                i = x * 6 + j
                for _ in range((i + 1) * npre // (6 * L) - i * npre // (6 * L)):
                    start(todo.pop(0), 0)
        start(xcp, 1)
        for g in range(T_BWQ):
            for j in range(6):
                for cp in low(streams[0], g, j):
                    cp.wait()
                if todo:
                    start(todo.pop(0), 0)
                start(low(owner(g + L), g + L, j), 1)
        with jax.named_scope('ph_idle') if scopes else contextlib.nullcontext():
            for cp in first + xcp:
                cp.wait()

        def q_body(g, c):
            for i in range(4):
                h = (g - T_BWQ) * 4 + i
                w = jnp.concatenate([wq_v[r * NH + h] for r in range(DM // 8)], axis=0)
                qa_s[pl.ds(h, NB, stride=NH), :] = jnp.dot(xa_v[...], w, preferred_element_type=F32)
                if i & 1:
                    yield c
        run(T_BWQ, T_WUK, "q", q_body)

        def head_pairs(w_v, t):
            for i in range(2):
                w = w_v.reshape(DM * pitch, DH)[pl.ds(2 * t + i, DM, stride=pitch), :]
                yield 4 * t + 2 * i, pltpu.bitcast(w << 16, F32).astype(BF16)
                yield 4 * t + 2 * i + 1, pltpu.bitcast(w & jnp.uint32(0xFFFF0000), F32).astype(BF16)

        def bq_body(g, c):
            for i, (h, w) in enumerate(head_pairs(bwq_v, g - T_WUK)):
                qb_s[h] = jnp.dot(xb_v[...], w, preferred_element_type=F32)
                if i & 1:
                    yield c
        run(T_WUK, T_C, "bq", bq_body)

        def abs_body(g, c):
            for i, (h, w) in enumerate(head_pairs(wuk_v, g - T_C)):
                r = lax.dot_general(qb_s[h].astype(BF16), w, NT, preferred_element_type=F32)
                for t in range(4):
                    qabs_s[t, pl.ds(h, NB, stride=NH), :] = r[:, t * 128:(t + 1) * 128]
                if i & 1:
                    yield c
        run(T_C, T_C + 8, "ab", abs_body)

        def lat_scores(t):
            r0 = pl.multiple_of((t >> 3) * NH, NH)
            q = jnp.concatenate([qabs_s[i, pl.ds(r0, NH), :] for i in range(4)], axis=1).astype(BF16)
            for i in range(2):
                keys = c_v[pl.ds(pl.multiple_of(t * 512 + i * 256, 256), 256), :]
                sb_s[:, i * 256:(i + 1) * 256] = lax.dot_general(q, keys, NT, preferred_element_type=F32) * SCALE
                yield

        def lat_body(g, carry):
            m, l = carry
            t = g - (T_C + 8)
            r0 = pl.multiple_of((t >> 3) * NH, NH)
            fresh = (t & 7) == 0
            m = jnp.where(fresh, -jnp.inf, m)
            s0 = sb_s[...]
            m_new = jnp.maximum(m, jnp.max(s0, axis=1, keepdims=True))
            alpha = jnp.exp(m - m_new)
            p = jnp.exp(s0 - m_new)
            l = jnp.where(fresh, 0.0, alpha * l) + jnp.sum(p, axis=1, keepdims=True)
            p = p.astype(BF16)
            for _ in lat_scores(jnp.minimum(t + 1, 31)):
                yield carry
            n = pn["lat"].split().count("c") - 2
            pv = 0
            for i in range(n):
                keys = c_v[pl.ds(pl.multiple_of(t * 512 + i * (512 // n), 256), 512 // n), :]
                pv = pv + jnp.dot(p[:, i * (512 // n):(i + 1) * (512 // n)], keys, preferred_element_type=F32)
                if i < n - 1:
                    yield carry
            norm = jnp.where((t & 7) == 7, 1.0 / l, 1.0)
            for i in range(4):
                acc = cc_s[i, pl.ds(r0, NH), :]
                cc_s[i, pl.ds(r0, NH), :] = (alpha * acc + pv[:, i * 128:(i + 1) * 128]) * norm
            yield m_new, l
        if only is None or "lat" in only:
            cc_s[...] = jnp.zeros(cc_s.shape, F32)
            list(lat_scores(0))
        run(T_C + 8, T_KV, "lat", lat_body, (jnp.zeros((NH, 1), F32), jnp.zeros((NH, 1), F32)))

        def ctx_body(g, c):
            for i, (h, w) in enumerate(head_pairs(wuv_v, g - T_KV)):
                cc = jnp.concatenate([cc_s[t, pl.ds(h, NB, stride=NH), :] for t in range(4)], axis=1)
                ob_s[h] = jnp.dot(cc.astype(BF16), w, preferred_element_type=F32)
                if i & 1:
                    yield c
        run(T_KV, T_KV + 8, "ctx", ctx_body)

        def kv_rows(ref, h, a, b):
            return pltpu.bitcast(ref[pl.ds(pl.multiple_of(h * 512 + a // 2, 64), (b - a) // 2), :], BF16)

        def kv_scores(i, a, b):
            h = (i * M) & 127
            q = jnp.broadcast_to(qa_s[pl.ds(h, 1), :], (8, DH)).astype(BF16)
            return lax.dot_general(q, kv_rows(k_v, h, a, b), NT, preferred_element_type=F32) * SCALE

        def kv_body(g, s0):
            i = g - (T_KV + 8)
            h = (i * M) & 127
            p = jnp.exp(s0 - jnp.max(s0, axis=1, keepdims=True))
            norm = 1.0 / jnp.sum(p, axis=1, keepdims=True)
            p = p.astype(BF16)
            parts = [[(0, WIN)] if k == WIN else [(0, k), (k, WIN)] for k in ksplit]
            s1 = []
            for a, b in parts[0]:
                s1.append(kv_scores(jnp.minimum(i + 1, 127), a, b))
                yield s0
            o = 0
            for a, b in parts[1]:
                o = o + jnp.dot(p[:, a:b], kv_rows(v_v, h, a, b), preferred_element_type=F32)
                if b < WIN:
                    yield s0
            oa_s[pl.ds(h, 1), :] = (o * norm)[0:1]
            yield jnp.concatenate(s1, axis=1)
        run(T_KV + 8, T_WO, "kv", kv_body, kv_scores(0, 0, WIN) if only is None or "kv" in only else 0)

        def project(o, w_v, h):
            return jnp.dot(o.astype(BF16), w_v[pl.ds(pl.multiple_of(h * DH, DH), DH), :], preferred_element_type=F32)

        def a_proj(t, i):
            h = ((t + 4 * (i & 1)) & 7) * 4 + 2 * (i & 1) + (i >> 1)
            return project(oa_s[pl.ds(h, NB, stride=NH), :], wo_v, h)

        def b_proj(yb, h0, n):
            for i in range(n):
                yb = yb + project(ob_s[h0 + i], bwo_v, h0 + i)
            return yb

        def out_first(g, yb):
            yb = b_proj(yb, 0, 4)
            yield yb
            yield b_proj(yb, 4, 4)

        def out_body(g, carry):
            ya, yb = carry
            t = g - (T_WO + 1)
            for i in range(4):
                ya = ya + a_proj(t, i)
            yield ya, yb
            yield ya, b_proj(yb, 8 + 6 * t, 6)

        def out_tail(g, ya):
            t = g - (T_WO + 1)
            for i in range(4):
                ya = ya + a_proj(t, i)
                if i & 1:
                    yield ya

        def out_last(g, ya):
            for i in range(4):
                ya = ya + a_proj(6, i)
            heads = [28, 14]
            o = [jnp.concatenate([oa_s[pl.ds(h + i, NB, stride=NH), :] for i in range(2)], axis=1) for h in heads]
            groups = [[(32, 64)], [(0, 32), (224, 32)], [(96, 64)], [(160, 64)]]
            lhs = [jnp.concatenate([o[s][:, r:r + n] for s in range(2) for r, n in grp], axis=1).astype(BF16)
                   for grp in groups]
            yield ya
            for x, grp in zip(lhs, groups):
                w = jnp.concatenate([wo_v[pl.ds(h * DH + r, n), :] for h in heads for r, n in grp], axis=0)
                ya = ya + jnp.dot(x, w, preferred_element_type=F32)
                yield ya

        z = jnp.zeros((NB, DM), F32)
        yb = run(T_WO, T_WO + 1, "o0", out_first, z)
        ya, yb = run(T_WO + 1, T_WO + 5, "out", out_body, (z, yb))
        dst = o_v if manual else o_ref
        dst[:, DM:2 * DM] = yb.astype(BF16)
        if manual == 2:
            cb = pltpu.make_async_copy(o_v.at[:, DM:2 * DM], o_ref.at[:, DM:2 * DM], x_sem.at[1])
            cb.start()
        ya = run(T_WO + 5, T_END - 1, "o2", out_tail, ya)
        ya = run(T_END - 1, T_END, "o1", out_last, ya)
        dst[:, 0:DM] = ya.astype(BF16)
        if manual:
            w = DM if manual == 2 else 2 * DM
            ca = pltpu.make_async_copy(o_v.at[:, 0:w], o_ref.at[:, 0:w], x_sem.at[0])
            ca.start()
            if manual == 2:
                cb.wait()
            ca.wait()

    @jax.jit
    def f(A_x, A_k_cache, A_v_cache, A_wq, A_wo, B_x, B_c_kv, B_w_q, B_w_uk, B_w_uv, B_w_o):
        vm = pltpu.VMEM
        wq = A_wq.reshape(DM // 8, 8, NH, DH).transpose(0, 2, 1, 3).reshape(DM // 8 * NH, 8, DH)
        out = pl.pallas_call(
            kern,
            out_shape=jax.ShapeDtypeStruct((NB, 2 * DM), BF16),
            in_specs=[pl.BlockSpec(memory_space=pl.ANY)] * 11,
            out_specs=pl.BlockSpec(memory_space=pl.ANY if manual else vm),
            scratch_shapes=[
                vm((NB, DM), BF16), vm((NB, DM), BF16),
                vm((NB * NH * WIN // 2, DH), U32), vm((NB * NH * WIN // 2, DH), U32),
                vm((DM // 8 * NH, 8, DH), BF16), vm((NH * DH, DM), BF16), vm((NB * SK, DM), BF16),
                vm((DM, pitch, DH), U32), vm((DM, pitch, DH), U32), vm((DM, pitch, DH), U32),
                vm((NH * DH, DM), BF16),
                vm((NB * NH, DH), F32), vm((NH, NB, DH), F32), vm((4, NB * NH, 128), F32),
                vm((NH, 512), F32), vm((4, NB * NH, 128), F32), vm((NB * NH, DH), F32), vm((NH, NB, DH), F32),
                vm((NB, 2 * DM), BF16),
                pltpu.SemaphoreType.DMA((RING * 6,)), pltpu.SemaphoreType.DMA((RING * 2,)), pltpu.SemaphoreType.DMA((3,)),
            ],
            compiler_params=pltpu.CompilerParams(vmem_limit_bytes=120 * 1024 * 1024, disable_bounds_checks=True,
                                                 disable_semaphore_checks=True, flags=flags),
        )(A_x.reshape(NB, DM), A_k_cache.reshape(-1, DH), A_v_cache.reshape(-1, DH), wq, A_wo,
          B_x.reshape(NB, DM), B_c_kv.reshape(-1, DM), B_w_q, B_w_uk, B_w_uv, B_w_o.reshape(-1, DM))
        return out.reshape(NB, 1, 2 * DM)
    return f


pallas_concat_heads__sliding_block_cached__compressed_kv_cla__decode_kernel = build(pat='ALL6')
```

```python
import functools

import jax
import jax.numpy as jnp
from jax import lax
from jax.experimental import pallas as pl
from jax.experimental.pallas import tpu as pltpu

F32, BF16, U32 = jnp.float32, jnp.bfloat16, jnp.uint32
NT = (((1,), (1,)), ((), ()))

NB, NH, DH, DM, SK = 4, 32, 128, 512, 4096
WIN = min(4096, max(256, SK // 4))
SCALE = DH**-0.5

T_WQ, T_BWQ, T_WUK, T_C, T_WUV, T_KV, T_BWO, T_WO, T_END = 0, 8, 16, 24, 56, 64, 192, 200, 208
AHEAD = 3
RING = AHEAD + 1
CUT_A, CUT_B = 32, 48
HEAD_HOP = 33
PITCH = 24

FLAT = (
    [(region, 0, 64) for region in range(6)],
    [(7, 0, 32), (7, 32, 16), (7, 48, 16), (6, 0, 32), (6, 32, 16), (6, 48, 16)],
)
WINDOW = (
    [((j % 2, j // 2 * 2), CUT_A + 64 * (j // 2), 64) for j in range(6)],
    [((0, 5), 0, 32), ((1, 5), 0, 16), ((1, 5), 16, 16), ((0, 5), 224, 32), ((1, 5), 224, 16), ((1, 5), 240, 16)],
)
LAST_SLOTS = {201: range(6), 202: range(6), 203: (0, 1, 3, 4), 204: (0, 1, 3, 4), 205: (0, 1, 3, 4)}


def _dot(a, b):
    return jnp.dot(a, b, preferred_element_type=F32)


def _dot_nt(a, b):
    return lax.dot_general(a, b, NT, preferred_element_type=F32)


def _kernel(xa_h, k_h, v_h, wq_h, wo_h, xb_h, c_h, bwq_h, wuk_h, wuv_h, bwo_h, o_ref,
            xa_v, xb_v, k_v, v_v, wq_v, wo_v, c_v, bwq_v, wuk_v, wuv_v, bwo_v,
            qa_s, oa_s, qb_s, qc_s, sc_s, cc_s, ob_s, low_sem, high_sem, once_sem):

    def dma(src, dst, src_row, dst_row, rows, align, sem):
        dst = dst.at[pl.ds(pl.multiple_of(dst_row, align), rows)]
        if dst.shape[1:] != src.shape[1:]:
            dst = dst.at[:, pl.ds(0, src.shape[1])]
        return pltpu.make_async_copy(src.at[pl.ds(pl.multiple_of(src_row, align), rows)], dst, sem)

    def flat(src, dst, unit, cut):
        def copies(t, piece, sem):
            region, off, size = piece
            first = region * 512 + cut + off
            room = 4096 - 7 * 64 - first
            parts = [(first, room), (first + room, size - room)] if 0 < room < size else [(first, size)]
            out = []
            for kib, n in parts:
                row = (t & 7) * (4 * unit) + kib // 16 * unit
                if kib + 7 * 64 >= 4096:
                    row = row & (256 * unit - 1)
                if src.shape[0] > 256 * unit:
                    row = row + (t & -8) * (32 * unit)
                out.append(dma(src, dst, row, row, n // 16 * unit, unit, sem))
            return out

        return copies

    def window(t, piece, sem):
        (side, lag), off, size = piece
        src, dst = ((k_h, k_v), (v_h, v_v))[side]
        head = (t * HEAD_HOP - lag * HEAD_HOP) & (NB * NH - 1)
        return [dma(src.bitcast(U32), dst, head * (SK // 2) + ((SK - WIN) // 2 + 2 * off),
                    head * (WIN // 2) + 2 * off, 2 * size, 32, sem)]

    streams = [
        (T_WQ, T_BWQ, flat(wq_h, wq_v, 8, CUT_A), FLAT),
        (T_BWQ, T_WUK, flat(bwq_h.bitcast(U32), bwq_v, 2, CUT_B), FLAT),
        (T_WUK, T_C, flat(wuk_h.bitcast(U32), wuk_v, 2, CUT_B), FLAT),
        (T_C, T_WUV, flat(c_h, c_v, 16, CUT_B), FLAT),
        (T_WUV, T_KV, flat(wuv_h.bitcast(U32), wuv_v, 2, CUT_B), FLAT),
        (T_KV, T_BWO, window, WINDOW),
        (T_BWO, T_WO, flat(bwo_h, bwo_v, 16, CUT_B), FLAT),
        (T_WO, T_END, flat(wo_h, wo_v, 16, CUT_A), FLAT),
    ]

    def stream_at(t):
        return next((s for s in streams if s[0] <= t < s[1]), None)

    def low(stream, t, j):
        first, _, copies, pieces = stream
        return copies(t - first, pieces[0][j], low_sem.at[(t & (RING - 1)) * 6 + j])

    def high(stream, t, j, sem=None):
        first, _, copies, pieces = stream
        sem = high_sem.at[(t & (RING - 1)) * 2 + j // 3] if sem is None else sem
        return copies(t - first, pieces[1][j], sem)

    def start(copies, priority):
        for copy in copies:
            copy.start(priority=priority)

    def wait(copies):
        for copy in copies:
            copy.wait()

    spread = [(t, j) for t in range(T_END - 4, T_END) for j in range(6)]

    def tick(due, ahead, work, t, carry):
        fired = set()

        def fire(j):
            if j in fired:
                return
            fired.add(j)
            if isinstance(t, int) and t > T_WO:
                if j in LAST_SLOTS.get(t, ()):
                    start(high(streams[-1], *spread.pop(0)), 0)
            else:
                start(high(ahead, t + AHEAD, j), 0)

        halves = work(t, carry, functools.partial(fire, 1))
        for j in range(6):
            wait(low(due, t, j))
            fire(j)
            if j % 3 == 0:
                for i in range(j, j + 3):
                    wait(high(due, t, i))
                carry = next(halves)
                if ahead is not None:
                    for i in range(j, j + 3):
                        start(low(ahead, t + AHEAD, i), 1)
        return carry

    def run(lo, hi, work, carry=0):
        cuts = sorted({lo, hi} | {s[1] - k for s in streams for k in (0, AHEAD) if lo < s[1] - k < hi})
        for a, b in zip(cuts, cuts[1:]):
            step = functools.partial(tick, stream_at(a), stream_at(a + AHEAD), work)
            carry = step(a, carry) if b == a + 1 else lax.fori_loop(a, b, step, carry)
        return carry

    x_copies = [pltpu.make_async_copy(xa_h, xa_v, once_sem.at[0]), pltpu.make_async_copy(xb_h, xb_v, once_sem.at[1])]
    todo = [high(stream_at(t), t, j, once_sem.at[2] if t < T_BWQ else None)
            for t in range(T_BWQ + AHEAD) for j in range(6)]
    wq_high = sum(todo[:6 * T_BWQ], [])
    for t in range(-AHEAD, T_BWQ):
        for j in range(6):
            if t >= 0:
                wait(low(stream_at(t), t, j))
                start(todo.pop(0), 0)
            start(low(stream_at(t + AHEAD), t + AHEAD, j), 1)
            if t < 0:
                start(todo.pop(0), 0)
        if t == -1:
            start(x_copies, 1)
    wait(wq_high + x_copies)

    def by_batch(head):
        return pl.ds(head, NB, stride=NH)

    def a_query(t, carry, midway):
        for i in range(4):
            head = (t - T_BWQ) * 4 + i
            w = jnp.concatenate([wq_v[r * NH + head] for r in range(DM // 8)], axis=0)
            qa_s[by_batch(head), :] = _dot(xa_v[...], w)
            if i % 2:
                yield carry

    def four_heads(w_v, t):
        for i in range(2):
            w = w_v.reshape(DM * PITCH, DH)[pl.ds(2 * t + i, DM, stride=PITCH), :]
            yield 4 * t + 2 * i, pltpu.bitcast(w << 16, F32).astype(BF16)
            yield 4 * t + 2 * i + 1, pltpu.bitcast(w & jnp.uint32(0xFFFF0000), F32).astype(BF16)

    def b_query(t, carry, midway):
        for i, (head, w) in enumerate(four_heads(bwq_v, t - T_WUK)):
            qb_s[head] = _dot(xb_v[...], w)
            if i % 2:
                yield carry

    def b_absorb(t, carry, midway):
        for i, (head, w) in enumerate(four_heads(wuk_v, t - T_C)):
            q = _dot_nt(qb_s[head].astype(BF16), w)
            for n in range(4):
                qc_s[n, by_batch(head), :] = q[:, n * 128:(n + 1) * 128]
            if i % 2:
                yield carry

    run(T_BWQ, T_WUK, a_query)
    run(T_WUK, T_C, b_query)
    run(T_C, T_C + 8, b_absorb)

    def batch_rows(block):
        return pl.ds(pl.multiple_of((block >> 3) * NH, NH), NH)

    def b_scores(block, midway):
        q = jnp.concatenate([qc_s[n, batch_rows(block), :] for n in range(4)], axis=1).astype(BF16)
        for i in range(2):
            keys = c_v[pl.ds(pl.multiple_of(block * 512 + i * 256, 256), 256), :]
            sc_s[:, i * 256:(i + 1) * 256] = _dot_nt(q, keys) * SCALE
            midway()

    def b_attend(t, carry, midway):
        block = t - (T_C + 8)
        fresh = (block & 7) == 0
        m_old = jnp.where(fresh, -jnp.inf, carry[0])
        s = sc_s[...]
        m = jnp.maximum(m_old, jnp.max(s, axis=1, keepdims=True))
        alpha = jnp.exp(m_old - m)
        p = jnp.exp(s - m)
        total = jnp.where(fresh, 0.0, alpha * carry[1]) + jnp.sum(p, axis=1, keepdims=True)
        p = p.astype(BF16)
        b_scores(jnp.minimum(block + 1, NB * 8 - 1), midway)
        yield carry
        pc = _dot(p, c_v[pl.ds(pl.multiple_of(block * 512, 512), 512), :])
        norm = jnp.where((block & 7) == 7, 1.0 / total, 1.0)
        for n in range(4):
            acc = cc_s[n, batch_rows(block), :]
            cc_s[n, batch_rows(block), :] = (alpha * acc + pc[:, n * 128:(n + 1) * 128]) * norm
        yield m, total

    def b_context(t, carry, midway):
        for i, (head, w) in enumerate(four_heads(wuv_v, t - T_KV)):
            latent = jnp.concatenate([cc_s[n, by_batch(head), :] for n in range(4)], axis=1)
            ob_s[head] = _dot(latent.astype(BF16), w)
            if i % 2:
                yield carry

    cc_s[...] = jnp.zeros(cc_s.shape, F32)
    b_scores(0, lambda: None)
    run(T_C + 8, T_KV, b_attend, (jnp.zeros((NH, 1), F32), jnp.zeros((NH, 1), F32)))
    run(T_KV, T_KV + 8, b_context)

    def cache(ref, head):
        return pltpu.bitcast(ref[pl.ds(pl.multiple_of(head * (WIN // 2), WIN // 2), WIN // 2), :], BF16)

    def a_scores(i):
        head = (i * HEAD_HOP) & (NB * NH - 1)
        q = jnp.broadcast_to(qa_s[pl.ds(head, 1), :], (8, DH)).astype(BF16)
        return _dot_nt(q, cache(k_v, head)) * SCALE

    def a_attend(t, s, midway):
        i = t - (T_KV + 8)
        head = (i * HEAD_HOP) & (NB * NH - 1)
        p = jnp.exp(s - jnp.max(s, axis=1, keepdims=True))
        norm = 1.0 / jnp.sum(p, axis=1, keepdims=True)
        p = p.astype(BF16)
        s_next = a_scores(jnp.minimum(i + 1, NB * NH - 1))
        yield s
        oa_s[pl.ds(head, 1), :] = (_dot(p, cache(v_v, head)) * norm)[0:1]
        yield s_next

    run(T_KV + 8, T_WO, a_attend, a_scores(0))

    def b_project(y, first, count):
        for head in range(first, first + count):
            y = y + _dot(ob_s[head].astype(BF16), bwo_v[pl.ds(head * DH, DH), :])
        return y

    def a_spans(page, regions):
        spans = []
        for region in regions:
            row = region * 512 + page * 64 + CUT_A
            end = row + 64
            while row < end:
                n = min(end - row, DH - row % DH)
                spans.append((row % (NH * DH), n))
                row += n
        return spans

    def a_inputs(page, regions):
        return jnp.concatenate([oa_s[by_batch(row // DH), :][:, row % DH:row % DH + n]
                                for row, n in a_spans(page, regions)], axis=1).astype(BF16)

    def a_project(page, regions, o=None):
        w = jnp.concatenate([wo_v[pl.ds(row, n), :] for row, n in a_spans(page, regions)], axis=0)
        return _dot(a_inputs(page, regions) if o is None else o, w)

    def project(t, carry, midway):
        ya, yb = carry
        page = t - T_WO
        if page == 0:
            yb = b_project(yb, 0, 4)
        else:
            ya = ya + a_project(page - 1, range(8) if page <= 5 else (4, 5))
        yield ya, yb
        if page == 0:
            yb = b_project(yb, 4, 4)
        elif page <= 4:
            yb = b_project(yb, 2 + 6 * page, 6)
        else:
            ya = ya + a_project(page, (0, 1, 2, 3, 6, 7))
        yield ya, yb

    ya = yb = jnp.zeros((NB, DM), F32)
    for t in range(T_WO, T_END - 1):
        ya, yb = run(t, t + 1, project, (ya, yb))
        if t == T_WO + 4:
            o_ref[:, DM:] = yb.astype(BF16)

    ya = ya + a_project(6, (4, 5))
    early, late = (0, 1, 2, 6, 7), (3, 4, 5)
    o_early, o_late = a_inputs(7, early), a_inputs(7, late)
    for j in range(3):
        wait(low(streams[-1], T_END - 1, j))
    for j in range(6):
        wait(high(streams[-1], T_END - 1, j))
    ya = ya + a_project(7, early, o_early)
    for j in late:
        wait(low(streams[-1], T_END - 1, j))
    ya = ya + a_project(7, late, o_late)
    o_ref[:, :DM] = ya.astype(BF16)


@jax.jit
def pallas_concat_heads__sliding_block_cached__compressed_kv_cla__decode_kernel(
    A_x: jax.Array,
    A_k_cache: jax.Array,
    A_v_cache: jax.Array,
    A_wq: jax.Array,
    A_wo: jax.Array,
    B_x: jax.Array,
    B_c_kv: jax.Array,
    B_w_q: jax.Array,
    B_w_uk: jax.Array,
    B_w_uv: jax.Array,
    B_w_o: jax.Array,
):
    assert A_x.shape == B_x.shape == (NB, 1, DM)
    assert A_k_cache.shape == A_v_cache.shape == (NB, NH, SK, DH)
    assert B_c_kv.shape == (NB, SK, DM)
    assert B_w_q.shape == B_w_uk.shape == B_w_uv.shape == (DM, NH, DH)
    vmem = pltpu.VMEM
    wq_tiles = A_wq.reshape(DM // 8, 8, NH, DH).transpose(0, 2, 1, 3).reshape(DM // 8 * NH, 8, DH)
    out = pl.pallas_call(
        _kernel,
        out_shape=jax.ShapeDtypeStruct((NB, 2 * DM), BF16),
        in_specs=[pl.BlockSpec(memory_space=pl.ANY)] * 11,
        out_specs=pl.BlockSpec(memory_space=vmem),
        scratch_shapes=[
            vmem((NB, DM), BF16),
            vmem((NB, DM), BF16),
            vmem((NB * NH * WIN // 2, DH), U32),
            vmem((NB * NH * WIN // 2, DH), U32),
            vmem((DM // 8 * NH, 8, DH), BF16),
            vmem((NH * DH, DM), BF16),
            vmem((NB * SK, DM), BF16),
            vmem((DM, PITCH, DH), U32),
            vmem((DM, PITCH, DH), U32),
            vmem((DM, PITCH, DH), U32),
            vmem((NH * DH, DM), BF16),
            vmem((NB * NH, DH), F32),
            vmem((NB * NH, DH), F32),
            vmem((NH, NB, DH), F32),
            vmem((4, NB * NH, 128), F32),
            vmem((NH, 512), F32),
            vmem((4, NB * NH, 128), F32),
            vmem((NH, NB, DH), F32),
            pltpu.SemaphoreType.DMA((RING * 6,)),
            pltpu.SemaphoreType.DMA((RING * 2,)),
            pltpu.SemaphoreType.DMA((3,)),
        ],
        compiler_params=pltpu.CompilerParams(
            vmem_limit_bytes=120 * 1024 * 1024,
            disable_bounds_checks=True,
            disable_semaphore_checks=True,
        ),
    )(
        A_x.reshape(NB, DM), A_k_cache.reshape(-1, DH), A_v_cache.reshape(-1, DH), wq_tiles, A_wo,
        B_x.reshape(NB, DM), B_c_kv.reshape(-1, DM), B_w_q, B_w_uk, B_w_uv, B_w_o.reshape(-1, DM),
    )
    return out.reshape(NB, 1, 2 * DM)
```

```python
import functools

import jax
import jax.numpy as jnp
from jax import lax
from jax.experimental import pallas as pl
from jax.experimental.pallas import tpu as pltpu

F32, BF16, U32 = jnp.float32, jnp.bfloat16, jnp.uint32
NT = (((1,), (1,)), ((), ()))

NB, NH, DH, DM, SK = 4, 32, 128, 512, 4096
WIN = min(4096, max(256, SK // 4))
SCALE = DH**-0.5

T_WQ, T_BWQ, T_WUK, T_C, T_KV, T_WUV, T_BWO, T_WO, T_END = 0, 8, 16, 24, 56, 184, 192, 200, 208
AHEAD = 3
RING = AHEAD + 1
CUT_A, CUT_B = 32, 48
HEAD_HOP = 33
PITCH = 516

FLAT = (
    [(region, 0, 64) for region in range(6)],
    [(7, 0, 32), (7, 32, 16), (7, 48, 16), (6, 0, 32), (6, 32, 16), (6, 48, 16)],
)
WINDOW = (
    [((j % 2, j // 2 * 2), CUT_A + 64 * (j // 2), 64) for j in range(6)],
    [((0, 5), 0, 32), ((1, 5), 0, 16), ((1, 5), 16, 16), ((0, 5), 224, 32), ((1, 5), 224, 16), ((1, 5), 240, 16)],
)
LAST_SLOTS = {201: range(6), 202: range(6), 203: (0, 1, 3, 4), 204: (0, 1, 3, 4), 205: (0, 1, 3, 4)}


def _dot(a, b):
    return jnp.dot(a, b, preferred_element_type=F32)


def _dot_nt(a, b):
    return lax.dot_general(a, b, NT, preferred_element_type=F32)


def _kernel(xa_h, k_h, v_h, wq_h, wo_h, xb_h, c_h, bwq_h, wuk_h, wuv_h, bwo_h, o_ref,
            xa_v, xb_v, k_v, v_v, wq_v, wo_v, c_v, bwq_v, wuk_v, wuv_v, bwo_v,
            pairs0_s, pairs1_s, qa_s, oa_s, qb_s, qc_s, sc_s, cc_s, ob_s, low_sem, high_sem, once_sem):

    def dma(src, dst, src_row, dst_row, rows, align, sem):
        return pltpu.make_async_copy(src.at[pl.ds(pl.multiple_of(src_row, align), rows)],
                                     dst.at[pl.ds(pl.multiple_of(dst_row, align), rows)], sem)

    def flat(src, dst, unit, cut):
        def copies(t, piece, sem):
            region, off, size = piece
            first = region * 512 + cut + off
            room = 4096 - 7 * 64 - first
            parts = [(first, room), (first + room, size - room)] if 0 < room < size else [(first, size)]
            out = []
            for kib, n in parts:
                row = (t & 7) * (4 * unit) + kib // 16 * unit
                if kib + 7 * 64 >= 4096:
                    row = row & (256 * unit - 1)
                if src.shape[0] > 256 * unit:
                    row = row + (t & -8) * (32 * unit)
                out.append(dma(src, dst, row, row, n // 16 * unit, unit, sem))
            return out

        return copies

    def window(t, piece, sem):
        (side, lag), off, size = piece
        src, dst = ((k_h, k_v), (v_h, v_v))[side]
        head = (t * HEAD_HOP - lag * HEAD_HOP) & (NB * NH - 1)
        return [dma(src, dst, head * SK + (SK - WIN + 4 * off), head * WIN + 4 * off, 4 * size, 64, sem)]

    streams = [
        (T_WQ, T_BWQ, flat(wq_h, wq_v, 8, CUT_A), FLAT),
        (T_BWQ, T_WUK, flat(bwq_h, bwq_v, 2, CUT_B), FLAT),
        (T_WUK, T_C, flat(wuk_h, wuk_v, 2, CUT_B), FLAT),
        (T_C, T_KV, flat(c_h, c_v, 16, CUT_B), FLAT),
        (T_KV, T_WUV, window, WINDOW),
        (T_WUV, T_BWO, flat(wuv_h, wuv_v, 2, CUT_B), FLAT),
        (T_BWO, T_WO, flat(bwo_h, bwo_v, 16, CUT_B), FLAT),
        (T_WO, T_END, flat(wo_h, wo_v, 16, CUT_A), FLAT),
    ]

    def stream_at(t):
        return next((s for s in streams if s[0] <= t < s[1]), None)

    def low(stream, t, j):
        first, _, copies, pieces = stream
        return copies(t - first, pieces[0][j], low_sem.at[(t & (RING - 1)) * 6 + j])

    def high(stream, t, j, sem=None):
        first, _, copies, pieces = stream
        sem = high_sem.at[(t & (RING - 1)) * 2 + j // 3] if sem is None else sem
        return copies(t - first, pieces[1][j], sem)

    def start(copies, priority):
        for copy in copies:
            copy.start(priority=priority)

    def wait(copies):
        for copy in copies:
            copy.wait()

    spread = [(t, j) for t in range(T_END - 4, T_END) for j in range(6)]

    def tick(due, ahead, work, t, carry):
        fired = set()

        def fire(j):
            if j in fired:
                return
            fired.add(j)
            if isinstance(t, int) and t > T_WO:
                if j in LAST_SLOTS.get(t, ()):
                    start(high(streams[-1], *spread.pop(0)), 0)
            else:
                start(high(ahead, t + AHEAD, j), 0)

        halves = work(t, carry, functools.partial(fire, 1))
        for j in range(6):
            wait(low(due, t, j))
            fire(j)
            if j % 3 == 0:
                for i in range(j, j + 3):
                    wait(high(due, t, i))
                carry = next(halves)
                if ahead is not None:
                    for i in range(j, j + 3):
                        start(low(ahead, t + AHEAD, i), 1)
        return carry

    def run(lo, hi, work, carry=0):
        cuts = sorted({lo, hi} | {s[1] - k for s in streams for k in (0, AHEAD) if lo < s[1] - k < hi})
        for a, b in zip(cuts, cuts[1:]):
            step = functools.partial(tick, stream_at(a), stream_at(a + AHEAD), work)
            carry = step(a, carry) if b == a + 1 else lax.fori_loop(a, b, step, carry)
        return carry

    x_copies = [pltpu.make_async_copy(xa_h, xa_v, once_sem.at[0]), pltpu.make_async_copy(xb_h, xb_v, once_sem.at[1])]
    todo = [high(stream_at(t), t, j, once_sem.at[2] if t < T_BWQ else None)
            for t in range(T_BWQ + AHEAD) for j in range(6)]
    wq_high = sum(todo[:6 * T_BWQ], [])
    for t in range(-AHEAD, T_BWQ):
        for j in range(6):
            if t >= 0:
                wait(low(stream_at(t), t, j))
                start(todo.pop(0), 0)
            start(low(stream_at(t + AHEAD), t + AHEAD, j), 1)
            if t < 0:
                start(todo.pop(0), 0)
        if t == -1:
            start(x_copies, 1)
    wait(wq_high + x_copies)

    def by_batch(head):
        return pl.ds(head, NB, stride=NH)

    def regroup(w_v, pairs_s, page, regions):
        for region in regions:
            for i in range(8):
                row = (page * 8 + (region * 64 + CUT_B // 8 + i)) & (DM - 1)
                pairs_s[pl.ds(row, NH // 2, stride=PITCH), :] = pltpu.bitcast(w_v[row], U32)

    def four_heads(pairs_s, t):
        for i in range(2):
            w = pairs_s[pl.ds((2 * t + i) * PITCH, DM), :]
            yield 4 * t + 2 * i, pltpu.bitcast(w << 16, F32).astype(BF16)
            yield 4 * t + 2 * i + 1, pltpu.bitcast(w & jnp.uint32(0xFFFF0000), F32).astype(BF16)

    def and_regroup(work, first, w_v, pairs_s):
        def both(t, carry, midway):
            halves = work(t, carry, midway)
            for regions in ((0, 7), (1, 2, 3, 6)):
                regroup(w_v, pairs_s, t - first, regions)
                yield next(halves)

        return both

    def regroup_rest(w_v, pairs_s):
        @pl.loop(0, 8)
        def _(page):
            regroup(w_v, pairs_s, page, (4, 5))

    def a_query(t, carry, midway):
        for i in range(4):
            head = (t - T_BWQ) * 4 + i
            w = jnp.concatenate([wq_v[r * NH + head] for r in range(DM // 8)], axis=0)
            qa_s[by_batch(head), :] = _dot(xa_v[...], w)
            if i % 2:
                yield carry

    def b_query(t, carry, midway):
        for i, (head, w) in enumerate(four_heads(pairs0_s, t - T_WUK)):
            qb_s[head] = _dot(xb_v[...], w)
            if i % 2:
                yield carry

    def b_absorb(t, carry, midway):
        for i, (head, w) in enumerate(four_heads(pairs1_s, t - T_C)):
            q = _dot_nt(qb_s[head].astype(BF16), w)
            for n in range(4):
                qc_s[n, by_batch(head), :] = q[:, n * 128:(n + 1) * 128]
            if i % 2:
                yield carry

    run(T_BWQ, T_WUK, and_regroup(a_query, T_BWQ, bwq_v, pairs0_s))
    regroup_rest(bwq_v, pairs0_s)
    run(T_WUK, T_C, and_regroup(b_query, T_WUK, wuk_v, pairs1_s))
    regroup_rest(wuk_v, pairs1_s)
    run(T_C, T_C + 8, b_absorb)

    def batch_rows(block):
        return pl.ds(pl.multiple_of((block >> 3) * NH, NH), NH)

    def b_scores(block, midway):
        q = jnp.concatenate([qc_s[n, batch_rows(block), :] for n in range(4)], axis=1).astype(BF16)
        for i in range(2):
            keys = c_v[pl.ds(pl.multiple_of(block * 512 + i * 256, 256), 256), :]
            sc_s[:, i * 256:(i + 1) * 256] = _dot_nt(q, keys) * SCALE
            midway()

    def b_attend(t, carry, midway):
        block = t - (T_C + 8)
        fresh = (block & 7) == 0
        m_old = jnp.where(fresh, -jnp.inf, carry[0])
        s = sc_s[...]
        m = jnp.maximum(m_old, jnp.max(s, axis=1, keepdims=True))
        alpha = jnp.exp(m_old - m)
        p = jnp.exp(s - m)
        total = jnp.where(fresh, 0.0, alpha * carry[1]) + jnp.sum(p, axis=1, keepdims=True)
        p = p.astype(BF16)
        b_scores(jnp.minimum(block + 1, NB * 8 - 1), midway)
        yield carry
        pc = _dot(p, c_v[pl.ds(pl.multiple_of(block * 512, 512), 512), :])
        norm = jnp.where((block & 7) == 7, 1.0 / total, 1.0)
        for n in range(4):
            acc = cc_s[n, batch_rows(block), :]
            cc_s[n, batch_rows(block), :] = (alpha * acc + pc[:, n * 128:(n + 1) * 128]) * norm
        yield m, total

    cc_s[...] = jnp.zeros(cc_s.shape, F32)
    b_scores(0, lambda: None)
    run(T_C + 8, T_KV + 8, b_attend, (jnp.zeros((NH, 1), F32), jnp.zeros((NH, 1), F32)))

    def cache(ref, head):
        return ref[pl.ds(pl.multiple_of(head * WIN, WIN), WIN), :]

    def a_scores(i):
        head = (i * HEAD_HOP) & (NB * NH - 1)
        q = jnp.broadcast_to(qa_s[pl.ds(head, 1), :], (8, DH)).astype(BF16)
        return _dot_nt(q, cache(k_v, head)) * SCALE

    def a_attend(t, s, midway):
        i = t - (T_KV + 8)
        head = (i * HEAD_HOP) & (NB * NH - 1)
        p = jnp.exp(s - jnp.max(s, axis=1, keepdims=True))
        norm = 1.0 / jnp.sum(p, axis=1, keepdims=True)
        p = p.astype(BF16)
        s_next = a_scores(jnp.minimum(i + 1, NB * NH - 1))
        yield s
        oa_s[pl.ds(head, 1), :] = (_dot(p, cache(v_v, head)) * norm)[0:1]
        yield s_next

    s = run(T_KV + 8, T_WUV, a_attend, a_scores(0))
    run(T_WUV, T_BWO, and_regroup(a_attend, T_WUV, wuv_v, pairs0_s), s)
    regroup_rest(wuv_v, pairs0_s)

    def b_context(t, carry, midway):
        for i, (head, w) in enumerate(four_heads(pairs0_s, t - T_BWO)):
            latent = jnp.concatenate([cc_s[n, by_batch(head), :] for n in range(4)], axis=1)
            ob_s[head] = _dot(latent.astype(BF16), w)
            if i % 2:
                yield carry

    run(T_BWO, T_WO, b_context)

    def b_project(y, first, count):
        for head in range(first, first + count):
            y = y + _dot(ob_s[head].astype(BF16), bwo_v[pl.ds(head * DH, DH), :])
        return y

    def a_spans(page, regions):
        spans = []
        for region in regions:
            row = region * 512 + page * 64 + CUT_A
            end = row + 64
            while row < end:
                n = min(end - row, DH - row % DH)
                spans.append((row % (NH * DH), n))
                row += n
        return spans

    def a_inputs(page, regions):
        return jnp.concatenate([oa_s[by_batch(row // DH), :][:, row % DH:row % DH + n]
                                for row, n in a_spans(page, regions)], axis=1).astype(BF16)

    def a_project(page, regions, o=None):
        w = jnp.concatenate([wo_v[pl.ds(row, n), :] for row, n in a_spans(page, regions)], axis=0)
        return _dot(a_inputs(page, regions) if o is None else o, w)

    def project(t, carry, midway):
        ya, yb = carry
        page = t - T_WO
        if page == 0:
            yb = b_project(yb, 0, 4)
        else:
            ya = ya + a_project(page - 1, range(8) if page <= 5 else (4, 5))
        yield ya, yb
        if page == 0:
            yb = b_project(yb, 4, 4)
        elif page <= 4:
            yb = b_project(yb, 2 + 6 * page, 6)
        else:
            ya = ya + a_project(page, (0, 1, 2, 3, 6, 7))
        yield ya, yb

    ya = yb = jnp.zeros((NB, DM), F32)
    for t in range(T_WO, T_END - 1):
        ya, yb = run(t, t + 1, project, (ya, yb))
        if t == T_WO + 4:
            o_ref[:, DM:] = yb.astype(BF16)

    ya = ya + a_project(6, (4, 5))
    early, late = (0, 1, 2, 6, 7), (3, 4, 5)
    o_early, o_late = a_inputs(7, early), a_inputs(7, late)
    for j in range(3):
        wait(low(streams[-1], T_END - 1, j))
    for j in range(6):
        wait(high(streams[-1], T_END - 1, j))
    ya = ya + a_project(7, early, o_early)
    for j in late:
        wait(low(streams[-1], T_END - 1, j))
    ya = ya + a_project(7, late, o_late)
    o_ref[:, :DM] = ya.astype(BF16)


@jax.jit
def pallas_concat_heads__sliding_block_cached__compressed_kv_cla__decode_kernel(
    A_x: jax.Array,
    A_k_cache: jax.Array,
    A_v_cache: jax.Array,
    A_wq: jax.Array,
    A_wo: jax.Array,
    B_x: jax.Array,
    B_c_kv: jax.Array,
    B_w_q: jax.Array,
    B_w_uk: jax.Array,
    B_w_uv: jax.Array,
    B_w_o: jax.Array,
):
    assert A_x.shape == B_x.shape == (NB, 1, DM)
    assert A_k_cache.shape == A_v_cache.shape == (NB, NH, SK, DH)
    assert B_c_kv.shape == (NB, SK, DM)
    assert B_w_q.shape == B_w_uk.shape == B_w_uv.shape == (DM, NH, DH)
    vmem = pltpu.VMEM
    wq_tiles = A_wq.reshape(DM // 8, 8, NH, DH).transpose(0, 2, 1, 3).reshape(DM // 8 * NH, 8, DH)
    out = pl.pallas_call(
        _kernel,
        out_shape=jax.ShapeDtypeStruct((NB, 2 * DM), BF16),
        in_specs=[pl.BlockSpec(memory_space=pl.ANY)] * 11,
        out_specs=pl.BlockSpec(memory_space=vmem),
        scratch_shapes=[
            vmem((NB, DM), BF16),
            vmem((NB, DM), BF16),
            vmem((NB * NH * WIN, DH), BF16),
            vmem((NB * NH * WIN, DH), BF16),
            vmem((DM // 8 * NH, 8, DH), BF16),
            vmem((NH * DH, DM), BF16),
            vmem((NB * SK, DM), BF16),
            vmem((DM, NH, DH), BF16),
            vmem((DM, NH, DH), BF16),
            vmem((DM, NH, DH), BF16),
            vmem((NH * DH, DM), BF16),
            vmem((NH // 2 * PITCH, DH), U32),
            vmem((NH // 2 * PITCH, DH), U32),
            vmem((NB * NH, DH), F32),
            vmem((NB * NH, DH), F32),
            vmem((NH, NB, DH), F32),
            vmem((4, NB * NH, 128), F32),
            vmem((NH, 512), F32),
            vmem((4, NB * NH, 128), F32),
            vmem((NH, NB, DH), F32),
            pltpu.SemaphoreType.DMA((RING * 6,)),
            pltpu.SemaphoreType.DMA((RING * 2,)),
            pltpu.SemaphoreType.DMA((3,)),
        ],
        compiler_params=pltpu.CompilerParams(
            vmem_limit_bytes=120 * 1024 * 1024,
            disable_bounds_checks=True,
            disable_semaphore_checks=True,
        ),
    )(
        A_x.reshape(NB, DM), A_k_cache.reshape(-1, DH), A_v_cache.reshape(-1, DH), wq_tiles, A_wo,
        B_x.reshape(NB, DM), B_c_kv.reshape(-1, DM), B_w_q, B_w_uk, B_w_uv, B_w_o.reshape(-1, DM),
    )
    return out.reshape(NB, 1, 2 * DM)
```

```python
import functools

import jax
import jax.numpy as jnp
from jax import lax
from jax.experimental import pallas as pl
from jax.experimental.pallas import tpu as pltpu

F32, BF16, U32 = jnp.float32, jnp.bfloat16, jnp.uint32
NT = (((1,), (1,)), ((), ()))

NB, NH, DH, DM, SK = 4, 32, 128, 512, 4096
WIN = min(4096, max(256, SK // 4))
SCALE = DH**-0.5

T_WQ, T_BWQ, T_WUK, T_C, T_KV, T_WUV, T_BWO, T_WO, T_END = 0, 8, 16, 24, 56, 184, 192, 200, 208
AHEAD = 3
RING = 4
CUT_A, CUT_B = 32, 48
PITCH = 516

FLAT = (
    [(region, 0, 64) for region in range(6)],
    [(7, 0, 32), (7, 32, 16), (7, 48, 16), (6, 0, 32), (6, 32, 16), (6, 48, 16)],
)
WINDOW = (
    [((j % 2, j // 2 * 2), CUT_A + 64 * (j // 2), 64) for j in range(6)],
    [((0, 5), 0, 32), ((1, 5), 0, 16), ((1, 5), 16, 16), ((0, 5), 224, 32), ((1, 5), 224, 16), ((1, 5), 240, 16)],
)
LAST_SLOTS = {201: range(6), 202: range(6), 203: (0, 1, 3, 4), 204: (0, 1, 3, 4), 205: (0, 1, 3, 4)}


def _dot(a, b):
    return jnp.dot(a, b, preferred_element_type=F32)


def _dot_nt(a, b):
    return lax.dot_general(a, b, NT, preferred_element_type=F32)


def _kernel(xa_h, k_h, v_h, wq_h, wo_h, xb_h, c_h, bwq_h, wuk_h, wuv_h, bwo_h, o_ref,
            xa_v, xb_v, k_v, v_v, wq_v, wo_v, c_v, bwq_v, wuk_v, wuv_v, bwo_v,
            pairs0_s, pairs1_s, qa_s, oa_s, qb_s, qc_s, sc_s, cc_s, ob_s, low_sem, high_sem, once_sem):

    def dma(src, dst, src_row, dst_row, rows, align, sem):
        return pltpu.make_async_copy(src.at[pl.ds(pl.multiple_of(src_row, align), rows)],
                                     dst.at[pl.ds(pl.multiple_of(dst_row, align), rows)], sem)

    def flat(src, dst, unit, cut):
        def copies(t, piece, sem):
            region, off, size = piece
            first = region * 512 + cut + off
            room = 4096 - 7 * 64 - first
            parts = [(first, room), (first + room, size - room)] if 0 < room < size else [(first, size)]
            out = []
            for kib, n in parts:
                row = (t & 7) * (4 * unit) + kib // 16 * unit
                if kib + 7 * 64 >= 4096:
                    row = row & (256 * unit - 1)
                if src.shape[0] > 256 * unit:
                    row = row + (t & -8) * (32 * unit)
                out.append(dma(src, dst, row, row, n // 16 * unit, unit, sem))
            return out

        return copies

    def window(t, piece, sem):
        (side, lag), off, size = piece
        src, dst = ((k_h, k_v), (v_h, v_v))[side]
        head = (t - lag) & (NB * NH - 1)
        return [dma(src, dst, head * SK + (SK - WIN + 4 * off), head * WIN + 4 * off, 4 * size, 64, sem)]

    streams = [
        (T_WQ, T_BWQ, flat(wq_h, wq_v, 8, CUT_A), FLAT),
        (T_BWQ, T_WUK, flat(bwq_h, bwq_v, 2, CUT_B), FLAT),
        (T_WUK, T_C, flat(wuk_h, wuk_v, 2, CUT_B), FLAT),
        (T_C, T_KV, flat(c_h, c_v, 16, CUT_B), FLAT),
        (T_KV, T_WUV, window, WINDOW),
        (T_WUV, T_BWO, flat(wuv_h, wuv_v, 2, CUT_B), FLAT),
        (T_BWO, T_WO, flat(bwo_h, bwo_v, 16, CUT_B), FLAT),
        (T_WO, T_END, flat(wo_h, wo_v, 16, CUT_A), FLAT),
    ]

    def stream_at(t):
        return next((s for s in streams if s[0] <= t < s[1]), None)

    def low(stream, t, j):
        first, _, copies, pieces = stream
        return copies(t - first, pieces[0][j], low_sem.at[(t & (RING - 1)) * 6 + j])

    def high(stream, t, j, sem=None):
        first, _, copies, pieces = stream
        sem = high_sem.at[(t & (RING - 1)) * 2 + j // 3] if sem is None else sem
        return copies(t - first, pieces[1][j], sem)

    def start(copies, priority):
        for copy in copies:
            copy.start(priority=priority)

    def wait(copies):
        for copy in copies:
            copy.wait()

    spread = [(t, j) for t in range(T_END - 4, T_END) for j in range(6)]

    def tick(due, ahead, work, t, carry):
        fired = set()

        def fire(j):
            if j in fired:
                return
            fired.add(j)
            if isinstance(t, int) and t > T_WO:
                if j in LAST_SLOTS.get(t, ()):
                    start(high(streams[-1], *spread.pop(0)), 0)
            else:
                start(high(ahead, t + AHEAD, j), 0)

        halves = work(t, carry, functools.partial(fire, 1))
        for j in range(6):
            wait(low(due, t, j))
            fire(j)
            if j % 3 == 0:
                for i in range(j, j + 3):
                    wait(high(due, t, i))
                carry = next(halves)
                if ahead is not None:
                    for i in range(j, j + 3):
                        start(low(ahead, t + AHEAD, i), 1)
        return carry

    def run(lo, hi, work, carry=0):
        cuts = sorted({lo, hi} | {s[1] - k for s in streams for k in (0, AHEAD) if lo < s[1] - k < hi})
        for a, b in zip(cuts, cuts[1:]):
            step = functools.partial(tick, stream_at(a), stream_at(a + AHEAD), work)
            carry = step(a, carry) if b == a + 1 else lax.fori_loop(a, b, step, carry)
        return carry

    x_copies = [pltpu.make_async_copy(xa_h, xa_v, once_sem.at[0]), pltpu.make_async_copy(xb_h, xb_v, once_sem.at[1])]
    todo = [high(stream_at(t), t, j, once_sem.at[2] if t < T_BWQ else None)
            for t in range(T_BWQ + AHEAD) for j in range(6)]
    wq_high = sum(todo[:6 * T_BWQ], [])
    for t in range(-AHEAD, T_BWQ):
        for j in range(6):
            if t >= 0:
                wait(low(stream_at(t), t, j))
                start(todo.pop(0), 0)
            start(low(stream_at(t + AHEAD), t + AHEAD, j), 1)
            if t < 0:
                start(todo.pop(0), 0)
        if t == -1:
            start(x_copies, 1)
    wait(wq_high + x_copies)

    def by_batch(head):
        return pl.ds(head, NB, stride=NH)

    def regroup(w_v, pairs_s, page, regions):
        for region in regions:
            for i in range(8):
                row = (page * 8 + (region * 64 + CUT_B // 8 + i)) & (DM - 1)
                pairs_s[pl.ds(row, NH // 2, stride=PITCH), :] = pltpu.bitcast(w_v[row], U32)

    def four_heads(pairs_s, t):
        for i in range(2):
            w = pairs_s[pl.ds((2 * t + i) * PITCH, DM), :]
            yield 4 * t + 2 * i, pltpu.bitcast(w << 16, F32).astype(BF16)
            yield 4 * t + 2 * i + 1, pltpu.bitcast(w & jnp.uint32(0xFFFF0000), F32).astype(BF16)

    def and_regroup(work, first, w_v, pairs_s):
        def both(t, carry, midway):
            halves = work(t, carry, midway)
            for regions in ((0, 7), (1, 2, 3, 6)):
                regroup(w_v, pairs_s, t - first, regions)
                yield next(halves)

        return both

    def regroup_rest(w_v, pairs_s):
        @pl.loop(0, 8)
        def _(page):
            regroup(w_v, pairs_s, page, (4, 5))

    def a_query(t, carry, midway):
        for i in range(4):
            head = (t - T_BWQ) * 4 + i
            w = jnp.concatenate([wq_v[r * NH + head] for r in range(DM // 8)], axis=0)
            qa_s[by_batch(head), :] = _dot(xa_v[...], w)
            if i % 2:
                yield carry

    def b_query(t, carry, midway):
        for i, (head, w) in enumerate(four_heads(pairs0_s, t - T_WUK)):
            qb_s[head] = _dot(xb_v[...], w)
            if i % 2:
                yield carry

    def b_absorb(t, carry, midway):
        for i, (head, w) in enumerate(four_heads(pairs1_s, t - T_C)):
            q = _dot_nt(qb_s[head].astype(BF16), w)
            for n in range(4):
                qc_s[n, by_batch(head), :] = q[:, n * 128:(n + 1) * 128]
            if i % 2:
                yield carry

    run(T_BWQ, T_WUK, and_regroup(a_query, T_BWQ, bwq_v, pairs0_s))
    regroup_rest(bwq_v, pairs0_s)
    run(T_WUK, T_C, and_regroup(b_query, T_WUK, wuk_v, pairs1_s))
    regroup_rest(wuk_v, pairs1_s)
    run(T_C, T_C + 8, b_absorb)

    def batch_rows(block):
        return pl.ds(pl.multiple_of((block >> 3) * NH, NH), NH)

    def b_scores(block, midway):
        q = jnp.concatenate([qc_s[n, batch_rows(block), :] for n in range(4)], axis=1).astype(BF16)
        for i in range(2):
            keys = c_v[pl.ds(pl.multiple_of(block * 512 + i * 256, 256), 256), :]
            sc_s[:, i * 256:(i + 1) * 256] = _dot_nt(q, keys) * SCALE
            midway()

    def b_attend(t, carry, midway):
        block = t - (T_C + 8)
        fresh = (block & 7) == 0
        m_old = jnp.where(fresh, -jnp.inf, carry[0])
        s = sc_s[...]
        m = jnp.maximum(m_old, jnp.max(s, axis=1, keepdims=True))
        alpha = jnp.exp(m_old - m)
        p = jnp.exp(s - m)
        total = jnp.where(fresh, 0.0, alpha * carry[1]) + jnp.sum(p, axis=1, keepdims=True)
        p = p.astype(BF16)
        b_scores(jnp.minimum(block + 1, NB * 8 - 1), midway)
        yield carry
        pc = _dot(p, c_v[pl.ds(pl.multiple_of(block * 512, 512), 512), :])
        norm = jnp.where((block & 7) == 7, 1.0 / total, 1.0)
        for n in range(4):
            acc = cc_s[n, batch_rows(block), :]
            cc_s[n, batch_rows(block), :] = (alpha * acc + pc[:, n * 128:(n + 1) * 128]) * norm
        yield m, total

    cc_s[...] = jnp.zeros(cc_s.shape, F32)
    b_scores(0, lambda: None)
    run(T_C + 8, T_KV + 8, b_attend, (jnp.zeros((NH, 1), F32), jnp.zeros((NH, 1), F32)))

    def cache(ref, head):
        return ref[pl.ds(pl.multiple_of(head * WIN, WIN), WIN), :]

    def a_scores(head):
        q = jnp.broadcast_to(qa_s[pl.ds(head, 1), :], (8, DH)).astype(BF16)
        return _dot_nt(q, cache(k_v, head)) * SCALE

    def a_attend(t, s, midway):
        head = t - (T_KV + 8)
        p = jnp.exp(s - jnp.max(s, axis=1, keepdims=True))
        norm = 1.0 / jnp.sum(p, axis=1, keepdims=True)
        p = p.astype(BF16)
        s_next = a_scores(jnp.minimum(head + 1, NB * NH - 1))
        yield s
        oa_s[pl.ds(head, 1), :] = (_dot(p, cache(v_v, head)) * norm)[0:1]
        yield s_next

    s = run(T_KV + 8, T_WUV, a_attend, a_scores(0))
    run(T_WUV, T_BWO, and_regroup(a_attend, T_WUV, wuv_v, pairs0_s), s)
    regroup_rest(wuv_v, pairs0_s)

    def b_context(t, carry, midway):
        for i, (head, w) in enumerate(four_heads(pairs0_s, t - T_BWO)):
            latent = jnp.concatenate([cc_s[n, by_batch(head), :] for n in range(4)], axis=1)
            ob_s[head] = _dot(latent.astype(BF16), w)
            if i % 2:
                yield carry

    run(T_BWO, T_WO, b_context)

    def b_project(y, first, count):
        for head in range(first, first + count):
            y = y + _dot(ob_s[head].astype(BF16), bwo_v[pl.ds(head * DH, DH), :])
        return y

    def a_spans(page, regions):
        spans = []
        for region in regions:
            row = region * 512 + page * 64 + CUT_A
            end = row + 64
            while row < end:
                n = min(end - row, DH - row % DH)
                spans.append((row % (NH * DH), n))
                row += n
        return spans

    def a_inputs(page, regions):
        return jnp.concatenate([oa_s[by_batch(row // DH), :][:, row % DH:row % DH + n]
                                for row, n in a_spans(page, regions)], axis=1).astype(BF16)

    def a_project(page, regions, o=None):
        w = jnp.concatenate([wo_v[pl.ds(row, n), :] for row, n in a_spans(page, regions)], axis=0)
        return _dot(a_inputs(page, regions) if o is None else o, w)

    def project(t, carry, midway):
        ya, yb = carry
        page = t - T_WO
        if page == 0:
            yb = b_project(yb, 0, 4)
        else:
            ya = ya + a_project(page - 1, range(8) if page <= 5 else (4, 5))
        yield ya, yb
        if page == 0:
            yb = b_project(yb, 4, 4)
        elif page <= 4:
            yb = b_project(yb, 2 + 6 * page, 6)
        else:
            ya = ya + a_project(page, (0, 1, 2, 3, 6, 7))
        yield ya, yb

    ya = yb = jnp.zeros((NB, DM), F32)
    for t in range(T_WO, T_END - 1):
        ya, yb = run(t, t + 1, project, (ya, yb))
        if t == T_WO + 4:
            o_ref[:, DM:] = yb.astype(BF16)

    ya = ya + a_project(6, (4, 5))
    early, late = (0, 1, 2, 6, 7), (3, 4, 5)
    o_early, o_late = a_inputs(7, early), a_inputs(7, late)
    for j in range(3):
        wait(low(streams[-1], T_END - 1, j))
    for j in range(6):
        wait(high(streams[-1], T_END - 1, j))
    ya = ya + a_project(7, early, o_early)
    for j in late:
        wait(low(streams[-1], T_END - 1, j))
    ya = ya + a_project(7, late, o_late)
    o_ref[:, :DM] = ya.astype(BF16)


@jax.jit
def pallas_concat_heads__sliding_block_cached__compressed_kv_cla__decode_kernel(
    A_x: jax.Array,
    A_k_cache: jax.Array,
    A_v_cache: jax.Array,
    A_wq: jax.Array,
    A_wo: jax.Array,
    B_x: jax.Array,
    B_c_kv: jax.Array,
    B_w_q: jax.Array,
    B_w_uk: jax.Array,
    B_w_uv: jax.Array,
    B_w_o: jax.Array,
):
    assert A_x.shape == B_x.shape == (NB, 1, DM)
    assert A_k_cache.shape == A_v_cache.shape == (NB, NH, SK, DH)
    assert B_c_kv.shape == (NB, SK, DM)
    assert B_w_q.shape == B_w_uk.shape == B_w_uv.shape == (DM, NH, DH)
    vmem = pltpu.VMEM
    wq_tiles = A_wq.reshape(DM // 8, 8, NH, DH).transpose(0, 2, 1, 3).reshape(DM // 8 * NH, 8, DH)
    out = pl.pallas_call(
        _kernel,
        out_shape=jax.ShapeDtypeStruct((NB, 2 * DM), BF16),
        in_specs=[pl.BlockSpec(memory_space=pl.ANY)] * 11,
        out_specs=pl.BlockSpec(memory_space=vmem),
        scratch_shapes=[
            vmem((NB, DM), BF16),
            vmem((NB, DM), BF16),
            vmem((NB * NH * WIN, DH), BF16),
            vmem((NB * NH * WIN, DH), BF16),
            vmem((DM // 8 * NH, 8, DH), BF16),
            vmem((NH * DH, DM), BF16),
            vmem((NB * SK, DM), BF16),
            vmem((DM, NH, DH), BF16),
            vmem((DM, NH, DH), BF16),
            vmem((DM, NH, DH), BF16),
            vmem((NH * DH, DM), BF16),
            vmem((NH // 2 * PITCH + DM, DH), U32),
            vmem((NH // 2 * PITCH + DM, DH), U32),
            vmem(((NB + 1) * NH, DH), F32),
            vmem(((NB + 1) * NH, DH), F32),
            vmem((NH, NB, DH), F32),
            vmem((4, (NB + 1) * NH, 128), F32),
            vmem((NH, 512), F32),
            vmem((4, (NB + 1) * NH, 128), F32),
            vmem((NH, NB, DH), F32),
            pltpu.SemaphoreType.DMA((RING * 6,)),
            pltpu.SemaphoreType.DMA((RING * 2,)),
            pltpu.SemaphoreType.DMA((3,)),
        ],
        compiler_params=pltpu.CompilerParams(
            vmem_limit_bytes=120 * 1024 * 1024,
            disable_bounds_checks=True,
            disable_semaphore_checks=True,
        ),
    )(
        A_x.reshape(NB, DM), A_k_cache.reshape(-1, DH), A_v_cache.reshape(-1, DH), wq_tiles, A_wo,
        B_x.reshape(NB, DM), B_c_kv.reshape(-1, DM), B_w_q, B_w_uk, B_w_uv, B_w_o.reshape(-1, DM),
    )
    return out.reshape(NB, 1, 2 * DM)
```

```python
import functools

import jax
import jax.numpy as jnp
from jax import lax
from jax.experimental import pallas as pl
from jax.experimental.pallas import tpu as pltpu

F32, BF16, U32 = jnp.float32, jnp.bfloat16, jnp.uint32
NT = (((1,), (1,)), ((), ()))

NB, NH, DH, DM, SK = 4, 32, 128, 512, 4096
WIN = min(4096, max(256, SK // 4))
SCALE = DH**-0.5

T_WQ, T_BWQ, T_WUK, T_C, T_KV, T_WUV, T_BWO, T_WO, T_END = 0, 8, 16, 24, 56, 184, 192, 200, 208
AHEAD = 3
RING = 4
CUT_A, CUT_B = 32, 48
PITCH = 516

FLAT = (
    [(region, 0, 64) for region in range(6)],
    [(7, 0, 32), (7, 32, 16), (7, 48, 16), (6, 0, 32), (6, 32, 16), (6, 48, 16)],
)
WINDOW = (
    [((j % 2, j // 2 * 2), 32 + 64 * (j // 2), 64) for j in range(6)],
    [((0, 5), 0, 32), ((1, 5), 0, 16), ((1, 5), 16, 16), ((0, 5), 224, 32), ((1, 5), 224, 16), ((1, 5), 240, 16)],
)
LAST_SLOTS = {201: range(6), 202: range(6), 203: (0, 1, 3, 4), 204: (0, 1, 3, 4), 205: (0, 1, 3, 4)}


def _dot(a, b):
    return jnp.dot(a, b, preferred_element_type=F32)


def _dot_nt(a, b):
    return lax.dot_general(a, b, NT, preferred_element_type=F32)


def _kernel(xa_h, k_h, v_h, wq_h, wo_h, xb_h, c_h, bwq_h, wuk_h, wuv_h, bwo_h, o_ref,
            xa_v, xb_v, k_v, v_v, wq_v, wo_v, c_v, bwq_v, wuk_v, wuv_v, bwo_v,
            pairs0_s, pairs1_s, qa_s, oa_s, qb_s, qc_s, sc_s, cc_s, ob_s, low_sem, high_sem, once_sem):

    def dma(src, dst, src_row, dst_row, rows, align, sem):
        return pltpu.make_async_copy(src.at[pl.ds(pl.multiple_of(src_row, align), rows)],
                                     dst.at[pl.ds(pl.multiple_of(dst_row, align), rows)], sem)

    def flat(src, dst, unit, cut):
        def copies(t, piece, sem):
            region, off, size = piece
            first = region * 512 + cut + off
            room = 4096 - 7 * 64 - first
            parts = [(first, room), (first + room, size - room)] if 0 < room < size else [(first, size)]
            out = []
            for kib, n in parts:
                row = (t & 7) * (4 * unit) + kib // 16 * unit
                if kib + 7 * 64 >= 4096:
                    row = row & (256 * unit - 1)
                if src.shape[0] > 256 * unit:
                    row = row + (t & -8) * (32 * unit)
                out.append(dma(src, dst, row, row, n // 16 * unit, unit, sem))
            return out

        return copies

    def window(t, piece, sem):
        (side, lag), off, size = piece
        src, dst = ((k_h, k_v), (v_h, v_v))[side]
        head = (t - lag) & (NB * NH - 1)
        return [dma(src, dst, head * SK + (SK - WIN + 4 * off), head * WIN + 4 * off, 4 * size, 64, sem)]

    streams = [
        (T_WQ, T_BWQ, flat(wq_h, wq_v, 8, CUT_A), FLAT),
        (T_BWQ, T_WUK, flat(bwq_h, bwq_v, 2, CUT_B), FLAT),
        (T_WUK, T_C, flat(wuk_h, wuk_v, 2, CUT_B), FLAT),
        (T_C, T_KV, flat(c_h, c_v, 16, CUT_B), FLAT),
        (T_KV, T_WUV, window, WINDOW),
        (T_WUV, T_BWO, flat(wuv_h, wuv_v, 2, CUT_B), FLAT),
        (T_BWO, T_WO, flat(bwo_h, bwo_v, 16, CUT_B), FLAT),
        (T_WO, T_END, flat(wo_h, wo_v, 16, CUT_A), FLAT),
    ]

    def stream_at(t):
        return next((s for s in streams if s[0] <= t < s[1]), None)

    def low(stream, t, j):
        first, _, copies, pieces = stream
        return copies(t - first, pieces[0][j], low_sem.at[(t & (RING - 1)) * 6 + j])

    def high(stream, t, j, sem=None):
        first, _, copies, pieces = stream
        sem = high_sem.at[(t & (RING - 1)) * 2 + j // 3] if sem is None else sem
        return copies(t - first, pieces[1][j], sem)

    def start(copies, priority):
        for copy in copies:
            copy.start(priority=priority)

    def wait(copies):
        for copy in copies:
            copy.wait()

    spread = [(t, j) for t in range(T_END - 4, T_END) for j in range(6)]

    def tick(due, ahead, work, t, carry):
        fired = set()

        def fire(j):
            if j in fired:
                return
            fired.add(j)
            if isinstance(t, int) and t > T_WO:
                if j in LAST_SLOTS.get(t, ()):
                    start(high(streams[-1], *spread.pop(0)), 0)
            else:
                start(high(ahead, t + AHEAD, j), 0)

        halves = work(t, carry, functools.partial(fire, 1))
        for j in range(6):
            wait(low(due, t, j))
            fire(j)
            if j % 3 == 0:
                for i in range(j, j + 3):
                    wait(high(due, t, i))
                carry = next(halves)
                if ahead is not None:
                    for i in range(j, j + 3):
                        start(low(ahead, t + AHEAD, i), 1)
        return carry

    def run(lo, hi, work, carry=0):
        cuts = sorted({lo, hi} | {s[1] - k for s in streams for k in (0, AHEAD) if lo < s[1] - k < hi})
        for a, b in zip(cuts, cuts[1:]):
            step = functools.partial(tick, stream_at(a), stream_at(a + AHEAD), work)
            carry = step(a, carry) if b == a + 1 else lax.fori_loop(a, b, step, carry)
        return carry

    x_copies = [pltpu.make_async_copy(xa_h, xa_v, once_sem.at[0]), pltpu.make_async_copy(xb_h, xb_v, once_sem.at[1])]
    todo = [streams[0][2](t, (region, off, 32), once_sem.at[2])
            for t in range(T_BWQ) for region in (7, 6) for off in (0, 32)]
    wq_high = sum(todo, [])
    todo += [high(streams[1], T_BWQ + t, j) for t in range(AHEAD) for j in range(6)]
    for t in range(-AHEAD, T_BWQ):
        for j in range(6):
            if t >= 0:
                wait(low(stream_at(t), t, j))
                start(todo.pop(0), 0)
            start(low(stream_at(t + AHEAD), t + AHEAD, j), 1)
            if (t, j) in ((-2, 0), (-1, 5)):
                start(todo.pop(0), 0)
        if t == -1:
            start(x_copies, 1)
    wait(wq_high + x_copies)

    def by_batch(head):
        return pl.ds(head, NB, stride=NH)

    def regroup(w_v, pairs_s, page, regions):
        for region in regions:
            for i in range(8):
                row = (page * 8 + (region * 64 + CUT_B // 8 + i)) & (DM - 1)
                pairs_s[pl.ds(row, NH // 2, stride=PITCH), :] = pltpu.bitcast(w_v[row], U32)

    def four_heads(pairs_s, t):
        for i in range(2):
            w = pairs_s[pl.ds((2 * t + i) * PITCH, DM), :]
            yield 4 * t + 2 * i, pltpu.bitcast(w << 16, F32).astype(BF16)
            yield 4 * t + 2 * i + 1, pltpu.bitcast(w & jnp.uint32(0xFFFF0000), F32).astype(BF16)

    def and_regroup(work, first, w_v, pairs_s):
        def both(t, carry, midway):
            halves = work(t, carry, midway)
            for regions in ((0, 7), (1, 2, 3, 6)):
                regroup(w_v, pairs_s, t - first, regions)
                yield next(halves)

        return both

    def regroup_rest(w_v, pairs_s):
        @pl.loop(0, 8)
        def _(page):
            regroup(w_v, pairs_s, page, (4, 5))

    def a_query(t, carry, midway):
        for i in range(4):
            head = (t - T_BWQ) * 4 + i
            w = jnp.concatenate([wq_v[r * NH + head] for r in range(DM // 8)], axis=0)
            qa_s[by_batch(head), :] = _dot(xa_v[...], w)
            if i % 2:
                yield carry

    def b_query(t, carry, midway):
        for i, (head, w) in enumerate(four_heads(pairs0_s, t - T_WUK)):
            qb_s[head] = _dot(xb_v[...], w)
            if i % 2:
                yield carry

    def b_absorb(t, carry, midway):
        for i, (head, w) in enumerate(four_heads(pairs1_s, t - T_C)):
            q = _dot_nt(qb_s[head].astype(BF16), w)
            for n in range(4):
                qc_s[n, by_batch(head), :] = q[:, n * 128:(n + 1) * 128]
            if i % 2:
                yield carry

    run(T_BWQ, T_WUK, and_regroup(a_query, T_BWQ, bwq_v, pairs0_s))
    regroup_rest(bwq_v, pairs0_s)
    run(T_WUK, T_C, and_regroup(b_query, T_WUK, wuk_v, pairs1_s))
    regroup_rest(wuk_v, pairs1_s)
    run(T_C, T_C + 8, b_absorb)

    def batch_rows(block):
        return pl.ds(pl.multiple_of((block >> 3) * NH, NH), NH)

    def b_scores(block, midway):
        q = jnp.concatenate([qc_s[n, batch_rows(block), :] for n in range(4)], axis=1).astype(BF16)
        for i in range(2):
            keys = c_v[pl.ds(pl.multiple_of(block * 512 + i * 256, 256), 256), :]
            sc_s[:, i * 256:(i + 1) * 256] = _dot_nt(q, keys) * SCALE
            midway()

    def b_attend(t, carry, midway):
        block = t - (T_C + 8)
        fresh = (block & 7) == 0
        m_old = jnp.where(fresh, -jnp.inf, carry[0])
        s = sc_s[...]
        m = jnp.maximum(m_old, jnp.max(s, axis=1, keepdims=True))
        alpha = jnp.exp(m_old - m)
        p = jnp.exp(s - m)
        total = jnp.where(fresh, 0.0, alpha * carry[1]) + jnp.sum(p, axis=1, keepdims=True)
        p = p.astype(BF16)
        b_scores(jnp.minimum(block + 1, NB * 8 - 1), midway)
        yield carry
        pc = _dot(p, c_v[pl.ds(pl.multiple_of(block * 512, 512), 512), :])
        norm = jnp.where((block & 7) == 7, 1.0 / total, 1.0)
        for n in range(4):
            acc = cc_s[n, batch_rows(block), :]
            cc_s[n, batch_rows(block), :] = (alpha * acc + pc[:, n * 128:(n + 1) * 128]) * norm
        yield m, total

    cc_s[...] = jnp.zeros(cc_s.shape, F32)
    b_scores(0, lambda: None)
    run(T_C + 8, T_KV + 8, b_attend, (jnp.zeros((NH, 1), F32), jnp.zeros((NH, 1), F32)))

    def cache(ref, head):
        return ref[pl.ds(pl.multiple_of(head * WIN, WIN), WIN), :]

    def a_scores(head):
        q = jnp.broadcast_to(qa_s[pl.ds(head, 1), :], (8, DH)).astype(BF16)
        return _dot_nt(q, cache(k_v, head)) * SCALE

    def a_attend(t, s, midway):
        head = t - (T_KV + 8)
        p = jnp.exp(s - jnp.max(s, axis=1, keepdims=True))
        norm = 1.0 / jnp.sum(p, axis=1, keepdims=True)
        p = p.astype(BF16)
        s_next = a_scores(jnp.minimum(head + 1, NB * NH - 1))
        yield s
        oa_s[pl.ds(head, 1), :] = (_dot(p, cache(v_v, head)) * norm)[0:1]
        yield s_next

    s = run(T_KV + 8, T_WUV, a_attend, a_scores(0))
    run(T_WUV, T_BWO, and_regroup(a_attend, T_WUV, wuv_v, pairs0_s), s)
    regroup_rest(wuv_v, pairs0_s)

    def b_context(t, carry, midway):
        for i, (head, w) in enumerate(four_heads(pairs0_s, t - T_BWO)):
            latent = jnp.concatenate([cc_s[n, by_batch(head), :] for n in range(4)], axis=1)
            ob_s[head] = _dot(latent.astype(BF16), w)
            if i % 2:
                yield carry

    run(T_BWO, T_WO, b_context)

    def b_project(y, first, count):
        for head in range(first, first + count):
            y = y + _dot(ob_s[head].astype(BF16), bwo_v[pl.ds(head * DH, DH), :])
        return y

    def a_spans(page, regions):
        spans = []
        for region in regions:
            row = region * 512 + page * 64 + CUT_A
            end = row + 64
            while row < end:
                n = min(end - row, DH - row % DH)
                spans.append((row % (NH * DH), n))
                row += n
        return spans

    def a_inputs(page, regions):
        return jnp.concatenate([oa_s[by_batch(row // DH), :][:, row % DH:row % DH + n]
                                for row, n in a_spans(page, regions)], axis=1).astype(BF16)

    def a_project(page, regions, o=None):
        w = jnp.concatenate([wo_v[pl.ds(row, n), :] for row, n in a_spans(page, regions)], axis=0)
        return _dot(a_inputs(page, regions) if o is None else o, w)

    def project(t, carry, midway):
        ya, yb = carry
        page = t - T_WO
        if page == 0:
            yb = b_project(yb, 0, 4)
        else:
            ya = ya + a_project(page - 1, range(8) if page <= 5 else (4, 5))
        yield ya, yb
        if page == 0:
            yb = b_project(yb, 4, 4)
        elif page <= 4:
            yb = b_project(yb, 2 + 6 * page, 6)
        else:
            ya = ya + a_project(page, (0, 1, 2, 3, 6, 7))
        yield ya, yb

    ya = yb = jnp.zeros((NB, DM), F32)
    for t in range(T_WO, T_END - 1):
        ya, yb = run(t, t + 1, project, (ya, yb))
        if t == T_WO + 4:
            o_ref[:, DM:] = yb.astype(BF16)

    ya = ya + a_project(6, (4, 5))
    early, late = (0, 1, 2, 6, 7), (3, 4, 5)
    o_early, o_late = a_inputs(7, early), a_inputs(7, late)
    for j in range(3):
        wait(low(streams[-1], T_END - 1, j))
    for j in range(6):
        wait(high(streams[-1], T_END - 1, j))
    ya = ya + a_project(7, early, o_early)
    for j in late:
        wait(low(streams[-1], T_END - 1, j))
    ya = ya + a_project(7, late, o_late)
    o_ref[:, :DM] = ya.astype(BF16)


@jax.jit
def pallas_concat_heads__sliding_block_cached__compressed_kv_cla__decode_kernel(
    A_x: jax.Array,
    A_k_cache: jax.Array,
    A_v_cache: jax.Array,
    A_wq: jax.Array,
    A_wo: jax.Array,
    B_x: jax.Array,
    B_c_kv: jax.Array,
    B_w_q: jax.Array,
    B_w_uk: jax.Array,
    B_w_uv: jax.Array,
    B_w_o: jax.Array,
):
    assert A_x.shape == B_x.shape == (NB, 1, DM)
    assert A_k_cache.shape == A_v_cache.shape == (NB, NH, SK, DH)
    assert B_c_kv.shape == (NB, SK, DM)
    assert B_w_q.shape == B_w_uk.shape == B_w_uv.shape == (DM, NH, DH)
    vmem = pltpu.VMEM
    wq_tiles = A_wq.reshape(DM // 8, 8, NH, DH).transpose(0, 2, 1, 3).reshape(DM // 8 * NH, 8, DH)
    out = pl.pallas_call(
        _kernel,
        out_shape=jax.ShapeDtypeStruct((NB, 2 * DM), BF16),
        in_specs=[pl.BlockSpec(memory_space=pl.ANY)] * 11,
        out_specs=pl.BlockSpec(memory_space=vmem),
        scratch_shapes=[
            vmem((NB, DM), BF16),
            vmem((NB, DM), BF16),
            vmem((NB * NH * WIN, DH), BF16),
            vmem((NB * NH * WIN, DH), BF16),
            vmem((DM // 8 * NH, 8, DH), BF16),
            vmem((NH * DH, DM), BF16),
            vmem((NB * SK, DM), BF16),
            vmem((DM, NH, DH), BF16),
            vmem((DM, NH, DH), BF16),
            vmem((DM, NH, DH), BF16),
            vmem((NH * DH, DM), BF16),
            vmem((NH // 2 * PITCH + DM, DH), U32),
            vmem((NH // 2 * PITCH + DM, DH), U32),
            vmem(((NB + 1) * NH, DH), F32),
            vmem(((NB + 1) * NH, DH), F32),
            vmem((NH, NB, DH), F32),
            vmem((4, (NB + 1) * NH, 128), F32),
            vmem((NH, 512), F32),
            vmem((4, (NB + 1) * NH, 128), F32),
            vmem((NH, NB, DH), F32),
            pltpu.SemaphoreType.DMA((RING * 6,)),
            pltpu.SemaphoreType.DMA((RING * 2,)),
            pltpu.SemaphoreType.DMA((3,)),
        ],
        compiler_params=pltpu.CompilerParams(
            vmem_limit_bytes=120 * 1024 * 1024,
            disable_bounds_checks=True,
            disable_semaphore_checks=True,
        ),
    )(
        A_x.reshape(NB, DM), A_k_cache.reshape(-1, DH), A_v_cache.reshape(-1, DH), wq_tiles, A_wo,
        B_x.reshape(NB, DM), B_c_kv.reshape(-1, DM), B_w_q, B_w_uk, B_w_uv, B_w_o.reshape(-1, DM),
    )
    return out.reshape(NB, 1, 2 * DM)
```
